```python
import jax
import jax.numpy as jnp

def _softmax(x, axis=-1):
    return jax.nn.softmax(x, axis=axis)

def _gelu(x):
    return jax.nn.gelu(x, approximate=True)

def _silu(x):
    return jax.nn.silu(x)

def _sigmoid(x):
    return jax.nn.sigmoid(x)

def _layernorm(x, axis=-1, eps=1e-05):
    m = jnp.mean(x, axis=axis, keepdims=True)
    v = jnp.var(x, axis=axis, keepdims=True)
    return (x - m) / jnp.sqrt(v + eps)

def _scatter_add(tgt, idx, src, axis=0):
    return tgt.at[idx].add(src)

def _segment_sum(src, seg, n):
    return jax.ops.segment_sum(src, seg, n)

class _Rng:

    def __init__(self, key):
        self._k = key

    def _next(self):
        self._k, sub = jax.random.split(self._k)
        return sub

    def normal(self, shape):
        return jax.random.normal(self._next(), shape, dtype=jnp.bfloat16)

    def randint(self, lo, hi, shape):
        return jax.random.randint(self._next(), shape, lo, hi, dtype=jnp.int32)

    def uniform(self, shape, lo=0.0, hi=1.0):
        return jax.random.uniform(self._next(), shape, jnp.bfloat16, lo, hi)

    def permutation(self, n):
        return jax.random.permutation(self._next(), n)
kernel_name = 'concat_heads__memory_aug_recurrent_mem_tr__compressed_kv_cla__prompt'

def setup_inputs():
    _rng = _Rng(jax.random.key(int.from_bytes(__import__("os").urandom(4), "little")))
    _w = lambda a: (lambda t: t.astype(jnp.bfloat16) if jnp.issubdtype(t.dtype, jnp.floating) else t)(jnp.asarray(a))

    def _A_setup():
        B, S, Dm = (1, 2048, 448)
        H, Dh = (16, 256)
        M, seg = (8, 32)
        seg = min(seg, S)
        S = S // seg * seg
        return {'x': _w((lambda *s: _rng.normal(s) * 0.05)(B, S, Dm)), 'mem0': _w((lambda *s: _rng.normal(s) * 0.05)(B, M, Dm)), 'Wq': _w((lambda *s: _rng.normal(s) * 0.05)(Dm, H, Dh) * Dm ** (-0.5)), 'Wk': _w((lambda *s: _rng.normal(s) * 0.05)(Dm, H, Dh) * Dm ** (-0.5)), 'Wv': _w((lambda *s: _rng.normal(s) * 0.05)(Dm, H, Dh) * Dm ** (-0.5)), 'Wo': _w((lambda *s: _rng.normal(s) * 0.05)(H, Dh, Dm) * (H * Dh) ** (-0.5)), 'seg_len': seg}
    _A_in = _A_setup()

    def _B_setup():
        B, H, Sq, Sk, D, M = (1, 16, 2048, 2048, 256, 448)
        Dc = 4 * D
        return {'x': _w((lambda *s: _rng.normal(s) * 0.05)(B, Sq, M)), 'c_kv': _w((lambda *s: _rng.normal(s) * 0.05)(B, Sk, Dc)), 'w_q': _w((lambda *s: _rng.normal(s) * 0.05)(M, H, D) * M ** (-0.5)), 'w_uk': _w((lambda *s: _rng.normal(s) * 0.05)(Dc, H, D) * Dc ** (-0.5)), 'w_uv': _w((lambda *s: _rng.normal(s) * 0.05)(Dc, H, D) * Dc ** (-0.5)), 'w_o': _w((lambda *s: _rng.normal(s) * 0.05)(H, D, M) * (H * D) ** (-0.5))}
    _B_in = _B_setup()
    return {'A_x': _A_in['x'], 'A_mem0': _A_in['mem0'], 'A_Wq': _A_in['Wq'], 'A_Wk': _A_in['Wk'], 'A_Wv': _A_in['Wv'], 'A_Wo': _A_in['Wo'], 'A_seg_len': _A_in['seg_len'], 'B_x': _B_in['x'], 'B_c_kv': _B_in['c_kv'], 'B_w_q': _B_in['w_q'], 'B_w_uk': _B_in['w_uk'], 'B_w_uv': _B_in['w_uv'], 'B_w_o': _B_in['w_o']}

def reference(A_x, A_mem0, A_Wq, A_Wk, A_Wv, A_Wo, A_seg_len, B_x, B_c_kv, B_w_q, B_w_uk, B_w_uv, B_w_o):

    def _A_ref(x, mem0, Wq, Wk, Wv, Wo, seg_len):
        B, S, Dm = x.shape
        H, Dh = (Wq.shape[1], Wq.shape[2])
        M = mem0.shape[1]
        scale = Dh ** (-0.5)
        n_seg = S // seg_len
        L = M + seg_len
        idx = jnp.arange(L)
        mask = (idx[:, None] < M) | (idx[:, None] >= idx[None, :])
        mem = mem0
        outs = []
        for s in range(n_seg):
            xs = x[:, s * seg_len:(s + 1) * seg_len, :].copy()
            h = jnp.concatenate([mem, xs], axis=1)
            q = jnp.einsum('btd,dhe->bhte', h, Wq)
            k = jnp.einsum('btd,dhe->bhte', h, Wk)
            v = jnp.einsum('btd,dhe->bhte', h, Wv)
            scores = jnp.einsum('bhqe,bhke->bhqk', q, k) * scale
            scores = jnp.where(mask[None, None], scores, -1000000000.0)
            p = _softmax(scores, axis=-1)
            o = jnp.einsum('bhqk,bhke->bhqe', p, v)
            o = jnp.einsum('bhte,hed->btd', o, Wo)
            mem = o[:, :M, :].copy()
            outs.append(o[:, M:, :])
        return jnp.concatenate(outs, axis=1)

    def _B_ref(x, c_kv, w_q, w_uk, w_uv, w_o):
        B, Sq, M = (x.shape[0], x.shape[1], x.shape[2])
        Sk = c_kv.shape[1]
        H, D = (w_q.shape[1], w_q.shape[2])
        q = jnp.einsum('bqm,mhd->bhqd', x, w_q)
        k = jnp.einsum('bkc,chd->bhkd', c_kv, w_uk)
        v = jnp.einsum('bkc,chd->bhkd', c_kv, w_uv)
        scores = jnp.einsum('bhqd,bhkd->bhqk', q, k) * D ** (-0.5)
        off = Sk - Sq
        qi = jnp.arange(Sq)[:, None]
        kj = jnp.arange(Sk)[None, :]
        cmask = kj <= qi + off
        scores = jnp.where(cmask[None, None], scores, -1000000000.0)
        p = _softmax(scores, axis=-1)
        ctx = jnp.einsum('bhqk,bhkd->bhqd', p, v)
        return jnp.einsum('bhqd,hdm->bqm', ctx, w_o)
    a = _A_ref(A_x, A_mem0, A_Wq, A_Wk, A_Wv, A_Wo, A_seg_len)
    b = _B_ref(B_x, B_c_kv, B_w_q, B_w_uk, B_w_uv, B_w_o)
    return jnp.concatenate([a, b], axis=-1)
```

```python
import functools
import jax
import jax.numpy as jnp
import numpy as np
from jax import lax
from jax.experimental import pallas as pl
from jax.experimental.pallas import tpu as pltpu

F32 = jnp.float32
BF16 = jnp.bfloat16
U32 = jnp.uint32
NEG = -1000000000.0

DO_A = True
DO_B = True
LAT_S = 150
LAT_O = 250
LAT_R = 120
LAT_M = 150
LAT_BP = 300
LAT_BO = 150
VERBOSE = False


def _dot(a, b):
    return lax.dot_general(a, b, (((1,), (0,)), ((), ())), preferred_element_type=F32)


def _dot_nt(a, b):
    return lax.dot_general(a, b, (((1,), (1,)), ((), ())), preferred_element_type=F32)


def _unpack(u, shift):
    w = (u << shift) & jnp.uint32(0xFFFF0000)
    return pltpu.bitcast(w, F32).astype(BF16)


class _Op:
    def __init__(self, name, cost, deps, fn):
        self.name, self.cost, self.deps, self.fn = name, cost, deps, fn
        self.end = None


def _merge(qa, qb):
    ta = sum(o.cost for o in qa) or 1
    tb = sum(o.cost for o in qb) or 1
    ia = ib = 0
    da = db = 0
    t = 0
    order = []
    stall = 0

    def ready(o):
        return max([0] + [d.end + lat for d, lat in o.deps])

    while ia < len(qa) or ib < len(qb):
        cand = []
        if ia < len(qa):
            cand.append((max(ready(qa[ia]), t), da / ta, 0))
        if ib < len(qb):
            cand.append((max(ready(qb[ib]), t), db / tb, 1))
        st, _, w = min(cand)
        o = qa[ia] if w == 0 else qb[ib]
        stall += st - t
        t = st + o.cost
        o.end = t
        order.append(o)
        if w == 0:
            ia += 1
            da += o.cost
        else:
            ib += 1
            db += o.cost
    if VERBOSE:
        print("sim total", t, "stall", stall)
        print(" ".join(o.name for o in order))
    return order


def _make_kernel(S, Dm, H, Dh, M, seg, Dc):
    n_seg = S // seg
    seg_per_head = n_seg // H
    L = M + seg
    BQ = 128
    nqb = S // BQ
    scale = Dh ** (-0.5)

    def kernel(xat_hbm, mem0_hbm, wq_hbm, wk_hbm, wv_hbm, wot_hbm,
               xbt_hbm, c_hbm, bwq_hbm, wuk_hbm, wuv_hbm, bwot_hbm,
               out_hbm,
               xat, xa, mem0, rq, rk, rv, wqkv, wot,
               xbt, xb, c, rbq, ruk, ruv, bwot,
               q_all, wtmp, wk_h, wv_h, kh, vh, acc, outa, outv, sems):

        def ucopy(src, dst, s0):
            su = src.bitcast(U32)
            return [pltpu.make_async_copy(su.at[:, :, pl.ds(128 * t, 128)], dst.at[t], sems.at[s0 + t])
                    for t in range(2)]

        cp_xb = [pltpu.make_async_copy(xbt_hbm, xbt, sems.at[0])]
        cp_bq = ucopy(bwq_hbm, rbq, 1)
        cp_c = [pltpu.make_async_copy(c_hbm, c, sems.at[3])]
        cp_uk = ucopy(wuk_hbm, ruk, 4)
        cp_uv = ucopy(wuv_hbm, ruv, 6)
        cp_a = (ucopy(wq_hbm, rq, 8) + ucopy(wk_hbm, rk, 10) + ucopy(wv_hbm, rv, 12)
                + [pltpu.make_async_copy(wot_hbm, wot, sems.at[14]),
                   pltpu.make_async_copy(xat_hbm, xat, sems.at[15]),
                   pltpu.make_async_copy(mem0_hbm, mem0, sems.at[16])])
        cp_bwo = [pltpu.make_async_copy(bwot_hbm, bwot, sems.at[17])]
        for cp in cp_xb + cp_bq + cp_c + cp_uk + cp_uv + cp_bwo + cp_a:
            cp.start()

        acc[...] = jnp.zeros(acc.shape, F32)

        for cp in cp_xb:
            cp.wait()
        xb[...] = xbt[...].T
        for cp in cp_bq:
            cp.wait()

        rbq2 = rbq.reshape(2 * Dm * 8, 128)

        def qproj(j, carry):
            for par in range(2):
                for t in range(2):
                    u = rbq2[pl.ds(t * Dm * 8 + j, Dm, stride=8), :]
                    wtmp[par, :, 128 * t:128 * (t + 1)] = _unpack(u, 16 * (1 - par))
            for par in range(2):
                q = _dot(xb[...], wtmp[par]) * scale
                q_all[2 * j + par] = q.astype(BF16)
            return carry

        lax.fori_loop(0, H // 2, qproj, 0)

        for cp in cp_c + cp_uk + cp_uv + cp_bwo:
            cp.wait()

        ruk2 = ruk.reshape(2 * Dc * 8, 128)
        ruv2 = ruv.reshape(2 * Dc * 8, 128)

        def unpack_kv(h):
            j = h // 2
            shift = (16 * (1 - h % 2)).astype(U32)
            for (r2, dst) in ((ruk2, wk_h), (ruv2, wv_h)):
                for t in range(2):
                    u = r2[pl.ds(t * Dc * 8 + j, Dc, stride=8), :]
                    dst[:, 128 * t:128 * (t + 1)] = _unpack(u, shift)

        unpack_kv(jnp.int32(0))

        row = lax.broadcasted_iota(jnp.int32, (BQ, BQ), 0)
        col = lax.broadcasted_iota(jnp.int32, (BQ, BQ), 1)
        cmask = col <= row
        arow = lax.broadcasted_iota(jnp.int32, (L, L), 0)
        acol = lax.broadcasted_iota(jnp.int32, (L, L), 1)
        amask = (arow < M) | (arow >= acol)

        def a_ops(s, st, prev):
            r0 = pl.multiple_of(s * seg, seg)
            v_ = {}

            def f_qk(hh):
                if hh == 0:
                    xs = xa[pl.ds(r0, seg), :].astype(F32)
                    v_["h"] = jnp.concatenate([st["mem"], xs], axis=0)
                hc = v_["h"]
                v_["q", hh] = _dot(hc, wqkv[:, hh * Dh:(hh + 1) * Dh]) * scale
                v_["k", hh] = _dot(hc, wqkv[:, (H + hh) * Dh:(H + hh + 1) * Dh]).astype(BF16)

            def f_v(hh):
                v_["v", hh] = _dot(v_["h"], wqkv[:, (2 * H + hh) * Dh:(2 * H + hh + 1) * Dh]).astype(BF16)

            def f_s(hh):
                sc = _dot_nt(v_.pop(("q", hh)), v_.pop(("k", hh)))
                sc = jnp.where(amask, sc, NEG)
                m = jnp.max(sc, axis=-1, keepdims=True)
                p = jnp.exp(sc - m)
                v_["p", hh] = p
                v_["r", hh] = 1.0 / jnp.sum(p, axis=-1, keepdims=True)

            def f_o(hh):
                v_["o", hh] = _dot(v_.pop(("p", hh)), v_.pop(("v", hh))) * v_.pop(("r", hh))

            def f_r(hh):
                d = _dot_nt(v_.pop(("o", hh)), wot[hh])
                v_["acc"] = d if hh == 0 else v_["acc"] + d
                if hh == H - 1:
                    outa[pl.ds(r0, seg), :] = v_["acc"][M:, :].astype(BF16)
                    st["mem"] = v_["acc"][:M, :]

            qk = [_Op("qk%d" % i, 160, [(prev, LAT_M)] if (i == 0 and prev) else [],
                      functools.partial(f_qk, i)) for i in range(H)]
            vv = [_Op("v%d" % i, 80, [], functools.partial(f_v, i)) for i in range(H)]
            ss = [_Op("s%d" % i, 20, [(qk[i], LAT_S)], functools.partial(f_s, i)) for i in range(H)]
            oo = [_Op("o%d" % i, 20, [(ss[i], LAT_O), (vv[i], LAT_S)], functools.partial(f_o, i)) for i in range(H)]
            rr = [_Op("r%d" % i, 80, [(oo[i], LAT_R)], functools.partial(f_r, i)) for i in range(H)]
            q = []
            for t in range(H + 3):
                if t < H:
                    q.append(qk[t])
                if 0 <= t - 1 < H:
                    q.append(ss[t - 1])
                    q.append(vv[t - 1])
                if 0 <= t - 2 < H:
                    q.append(oo[t - 2])
                if 0 <= t - 3 < H:
                    q.append(rr[t - 3])
            return q

        def b_ops(h):
            v_ = {}

            def f_qk(i):
                n = BQ * (i + 1)
                q = q_all[h, BQ * i:BQ * (i + 1), :]
                sc = _dot_nt(q, kh[0:n, :])
                sd = jnp.where(cmask, sc[:, n - BQ:], NEG)
                sc = jnp.concatenate([sc[:, :n - BQ], sd], axis=1) if i > 0 else sd
                m = jnp.max(sc, axis=-1, keepdims=True)
                p = jnp.exp(sc - m)
                v_["r", i] = 1.0 / jnp.sum(p, axis=-1, keepdims=True)
                v_["p", i] = p.astype(BF16)

            def f_pv(i):
                n = BQ * (i + 1)
                v_["c", i] = (_dot(v_.pop(("p", i)), vh[0:n, :]) * v_.pop(("r", i))).astype(BF16)

            def f_op(i):
                acc[BQ * i:BQ * (i + 1), :] += _dot_nt(v_.pop(("c", i)), bwot[h])

            qk = [_Op("QK%d" % i, 64 * (i + 1), [], functools.partial(f_qk, i)) for i in range(nqb)]
            pv = [_Op("PV%d" % i, 64 * (i + 1), [(qk[i], LAT_BP + 16 * (i + 1))], functools.partial(f_pv, i))
                  for i in range(nqb)]
            op = [_Op("OP%d" % i, 256, [(pv[i], LAT_BO)], functools.partial(f_op, i)) for i in range(nqb)]
            q = []
            for t in range(nqb + 2):
                for d, ops in enumerate((qk, pv, op)):
                    if 0 <= t - d < nqb:
                        q.append(ops[nqb - 1 - (t - d)])
            return q

        def head(h, mem):
            if DO_B:
                kh[...] = _dot(c[...], wk_h[...]).astype(BF16)
                vh[...] = _dot(c[...], wv_h[...]).astype(BF16)

            @pl.when(h == 0)
            def _():
                for cp in cp_a:
                    cp.wait()
                xa[...] = xat[...].T
                for wi, r in enumerate((rq, rk, rv)):
                    r2 = r.reshape(2 * Dm * 8, 128)

                    def unp(jj, carry):
                        for par in range(2):
                            for t in range(2):
                                u = r2[pl.ds(t * Dm * 8 + jj, Dm, stride=8), :]
                                c0 = pl.multiple_of(wi * H * Dh + (2 * jj + par) * Dh + 128 * t, 128)
                                wqkv[:, pl.ds(c0, 128)] = _unpack(u, 16 * (1 - par))
                        return carry
                    lax.fori_loop(0, H // 2, unp, 0)

            st = {"mem": jnp.where(h == 0, mem0[...].astype(F32), mem)}
            qa = []
            if DO_A:
                for t in range(seg_per_head):
                    qa += a_ops(h * seg_per_head + t, st, qa[-1] if qa else None)
            qb = b_ops(h) if DO_B else []
            if DO_B:
                unpack_kv(jnp.minimum(h + 1, H - 1))
            for o in _merge(qa, qb):
                o.fn()
            return st["mem"]

        lax.fori_loop(0, H, head, jnp.zeros((M, Dm), F32))

        outv[:, 0:Dm] = outa[...]
        outv[:, Dm:] = acc[...].astype(BF16)
        cp = pltpu.make_async_copy(outv, out_hbm, sems.at[18])
        cp.start()
        cp.wait()

    return kernel


@functools.partial(jax.jit, static_argnames=("A_seg_len",))
def pallas_concat_heads__memory_aug_recurrent_mem_tr__compressed_kv_cla__prompt_kernel(A_x, A_mem0, A_Wq, A_Wk, A_Wv, A_Wo, A_seg_len, B_x, B_c_kv, B_w_q, B_w_uk, B_w_uv, B_w_o):
    _, S, Dm = A_x.shape
    M = A_mem0.shape[1]
    H, Dh = A_Wq.shape[1], A_Wq.shape[2]
    Dc = B_c_kv.shape[2]
    seg = int(A_seg_len)
    kern = _make_kernel(S, Dm, H, Dh, M, seg, Dc)
    any_spec = pl.BlockSpec(memory_space=pl.ANY)
    scratch = [
        pltpu.VMEM((Dm, S), BF16),
        pltpu.VMEM((S, Dm), BF16),
        pltpu.VMEM((M, Dm), BF16),
        pltpu.VMEM((2, Dm, 8, 128), U32),
        pltpu.VMEM((2, Dm, 8, 128), U32),
        pltpu.VMEM((2, Dm, 8, 128), U32),
        pltpu.VMEM((Dm, 3 * H * Dh), BF16),
        pltpu.VMEM((H, Dm, Dh), BF16),
        pltpu.VMEM((Dm, S), BF16),
        pltpu.VMEM((S, Dm), BF16),
        pltpu.VMEM((S, Dc), BF16),
        pltpu.VMEM((2, Dm, 8, 128), U32),
        pltpu.VMEM((2, Dc, 8, 128), U32),
        pltpu.VMEM((2, Dc, 8, 128), U32),
        pltpu.VMEM((H, Dm, Dh), BF16),
        pltpu.VMEM((H, S, Dh), BF16),
        pltpu.VMEM((2, Dm, Dh), BF16),
        pltpu.VMEM((Dc, Dh), BF16),
        pltpu.VMEM((Dc, Dh), BF16),
        pltpu.VMEM((S, Dh), BF16),
        pltpu.VMEM((S, Dh), BF16),
        pltpu.VMEM((S, Dm), F32),
        pltpu.VMEM((S, Dm), BF16),
        pltpu.VMEM((S, 2 * Dm), BF16),
        pltpu.SemaphoreType.DMA((19,)),
    ]
    out = pl.pallas_call(
        kern,
        out_shape=jax.ShapeDtypeStruct((S, 2 * Dm), BF16),
        in_specs=[any_spec] * 12,
        out_specs=any_spec,
        scratch_shapes=scratch,
        compiler_params=pltpu.CompilerParams(vmem_limit_bytes=120 * 1024 * 1024),
    )(A_x[0].T, A_mem0.reshape(M, Dm), A_Wq, A_Wk, A_Wv, jnp.swapaxes(A_Wo, 1, 2),
      B_x[0].T, B_c_kv.reshape(S, Dc), B_w_q, B_w_uk, B_w_uv, jnp.swapaxes(B_w_o, 1, 2))
    return out.reshape(1, S, 2 * Dm)
```

```python
import functools
import jax
import jax.numpy as jnp
import numpy as np
from jax import lax
from jax.experimental import pallas as pl
from jax.experimental.pallas import tpu as pltpu

F32 = jnp.float32
BF16 = jnp.bfloat16
U32 = jnp.uint32
NEG = -1000000000.0

DO_A = True
DO_B = True
LAT_S = 250
LAT_O = 250
LAT_R = 120
LAT_M = 150
LAT_BP = 300
LAT_BO = 150
VERBOSE = False
LOG2E = 1.4426950408889634
OB = 256
BIAS = 0.04
KC = 256
RM = 32
RS = 16
KVC = 1024
EC = 128
LAT_BE = 150
ORDER = lambda n: list(range(n - 1, -1, -1))


def _dot(a, b):
    return lax.dot_general(a, b, (((1,), (0,)), ((), ())), preferred_element_type=F32)


def _dot_nt(a, b):
    return lax.dot_general(a, b, (((1,), (1,)), ((), ())), preferred_element_type=F32)


def _unpack(u, shift):
    w = (u << shift) & jnp.uint32(0xFFFF0000)
    return pltpu.bitcast(w, F32).astype(BF16)


def _ld(words):
    return pltpu.bitcast(words, BF16)


def _pk(x):
    return pltpu.bitcast(x.astype(BF16), U32)


class _Op:
    def __init__(self, name, cost, deps, fn):
        self.name, self.cost, self.deps, self.fn = name, cost, deps, fn
        self.end = None


def _merge(qa, qb):
    ta = sum(o.cost for o in qa) or 1
    tb = sum(o.cost for o in qb) or 1
    ia = ib = 0
    da = db = 0
    t = 0
    order = []
    stall = 0

    def ready(o):
        return max([0] + [d.end + lat for d, lat in o.deps])

    while ia < len(qa) or ib < len(qb):
        cand = []
        if ia < len(qa):
            cand.append((max(ready(qa[ia]), t), da / ta, 0))
        if ib < len(qb):
            cand.append((max(ready(qb[ib]), t), db / tb + BIAS, 1))
        st, _, w = min(cand)
        o = qa[ia] if w == 0 else qb[ib]
        stall += st - t
        t = st + o.cost
        o.end = t
        order.append(o)
        if w == 0:
            ia += 1
            da += o.cost
        else:
            ib += 1
            db += o.cost
    if VERBOSE:
        print("sim total", t, "stall", stall)
        print(" ".join(o.name for o in order))
    return order


def _make_kernel(S, Dm, H, Dh, M, seg, Dc):
    n_seg = S // seg
    seg_per_head = n_seg // H
    L = M + seg
    BQ = 128
    nqb = S // BQ
    scale = Dh ** (-0.5) * LOG2E
    PAD = (-Dm) % 128
    LO = Dm + PAD - 128

    def kernel(xat_hbm, mem0_hbm, wq_hbm, wk_hbm, wv_hbm, wot_hbm,
               xbt_hbm, c_hbm, bwq_hbm, wuk_hbm, wuv_hbm, bwot_hbm,
               out_hbm,
               xat, xa, mem0, rq, rk, rv, wqkv, wot,
               xbt, c, rbq, ruk, ruv, bwot,
               qt_all, memf, kh, vth, acct, outv, sems):

        NP = H // 2

        def pcopy(src, dst, j, s0):
            return pltpu.make_async_copy(src.bitcast(U32).at[:, j, :], dst.at[j], sems.at[s0, j])

        def q_copies(j):
            return [pcopy(bwq_hbm, rbq, j, 0)]

        def a_copies(j):
            return [pcopy(wq_hbm, rq, j, 1), pcopy(wk_hbm, rk, j, 2), pcopy(wv_hbm, rv, j, 3)]

        def kv_copies(j):
            return [pcopy(wuk_hbm, ruk, j, 4), pcopy(wuv_hbm, ruv, j, 5)]

        cp_x = pltpu.make_async_copy(xbt_hbm.bitcast(U32), xbt, sems.at[6, 0])
        cp_xa = pltpu.make_async_copy(xat_hbm, xat, sems.at[6, 1])
        cp_m = pltpu.make_async_copy(mem0_hbm, mem0, sems.at[6, 3])
        CR = S // NP // 2

        def rest_copies(j):
            r0 = pl.multiple_of(j * CR, CR)
            return [pltpu.make_async_copy(c_hbm.bitcast(U32).at[pl.ds(r0, CR)], c.at[pl.ds(r0, CR)], sems.at[8, j]),
                    pltpu.make_async_copy(wot_hbm.bitcast(U32).at[pl.ds(2 * j, 2)], wot.at[pl.ds(2 * j, 2)], sems.at[9, j]),
                    pltpu.make_async_copy(bwot_hbm.bitcast(U32).at[pl.ds(2 * j, 2)], bwot.at[pl.ds(2 * j, 2)], sems.at[10, j])]

        for cp in [cp_x] + q_copies(0) + a_copies(0) + [cp_xa, cp_m] + q_copies(1) + a_copies(1):
            cp.start()

        acct[...] = jnp.zeros(acct.shape, F32)
        with jax.named_scope('s_xwait'):
            cp_x.wait()

        def qproj(j, carry):
            for cp in q_copies(j):
                cp.wait()
            for cp in rest_copies(j):
                cp.start()

            @pl.when(j + 2 < NP)
            def _():
                for cp in q_copies(j + 2) + a_copies(j + 2):
                    cp.start()

            @pl.when(j + 2 == NP)
            def _():
                for cp in kv_copies(0):
                    cp.start()

            ut = rbq[j].T
            fill = []
            for wi, r in enumerate((rq, rk, rv)):
                for par in range(2):
                    def f(wi=wi, r=r, par=par):
                        c0 = pl.multiple_of(wi * H * Dh + (2 * j + par) * Dh, Dh)
                        wqkv[:, pl.ds(c0, Dh)] = _pk(_unpack(r[j], 16 * (1 - par)))
                    fill.append(f)

            def tr():
                n = S // NP
                r0 = pl.multiple_of(j * n, n)
                xa[pl.ds(pl.multiple_of(j * (n // 2), n // 2), n // 2), :] = _pk(xat[:, pl.ds(r0, n)].T)
            fill.append(tr)
            nchunk = 8
            cw = S // nchunk
            for par in range(2):
                wt = _unpack(ut, 16 * (1 - par))
                for n in range(nchunk):
                    qt_all[2 * j + par, :, n * cw:(n + 1) * cw] = _pk(
                        _dot(wt, _ld(xbt[:, n * cw:(n + 1) * cw])) * scale)
                    if par == 1 and fill:
                        fill.pop(0)()
                if par == 0:
                    for cp in a_copies(j):
                        cp.wait()

                    @pl.when(j == 0)
                    def _():
                        cp_xa.wait()
            return carry

        with jax.named_scope('s_qproj'):
            lax.fori_loop(0, NP, qproj, 0)

        with jax.named_scope('s_wait2'):
            for j in range(NP):
                for cp in rest_copies(j):
                    cp.wait()
            for cp in kv_copies(0) + [cp_m]:
                cp.wait()

        memf[...] = mem0[...].astype(F32)
        krow = lax.broadcasted_iota(jnp.int32, (BQ, BQ), 0)
        qcol = lax.broadcasted_iota(jnp.int32, (BQ, BQ), 1)
        cmask = krow <= qcol
        arow = lax.broadcasted_iota(jnp.int32, (L, L), 0)
        acol = lax.broadcasted_iota(jnp.int32, (L, L), 1)
        amask = (arow < M) | (arow >= acol)

        def a_ops(s, st, prev):
            r0 = pl.multiple_of(s * seg, seg)
            v_ = {}

            def f_qk(hh):
                if hh == 0:
                    xs = _ld(xa[pl.ds(pl.multiple_of(s * (seg // 2), seg // 2), seg // 2), :]).astype(F32)
                    v_["h"] = jnp.concatenate([st["mem"], xs], axis=0)
                hc = v_["h"]
                v_["q", hh] = _dot(hc, _ld(wqkv[:, hh * Dh:(hh + 1) * Dh])) * scale
                v_["k", hh] = _dot(hc, _ld(wqkv[:, (H + hh) * Dh:(H + hh + 1) * Dh])).astype(BF16)

            def f_v(hh):
                v_["v", hh] = _dot(v_["h"], _ld(wqkv[:, (2 * H + hh) * Dh:(2 * H + hh + 1) * Dh])).astype(BF16)

            def f_s(hh):
                sc = _dot_nt(v_.pop(("q", hh)), v_.pop(("k", hh)))
                sc = jnp.where(amask, sc, NEG)
                m = jnp.max(sc, axis=-1, keepdims=True)
                p = jnp.exp2(sc - m)
                v_["p", hh] = p
                v_["r", hh] = 1.0 / jnp.sum(p, axis=-1, keepdims=True)

            def f_o(hh):
                v_["o", hh] = _dot(v_.pop(("p", hh)), v_.pop(("v", hh))) * v_.pop(("r", hh))

            def f_r(hh):
                d = _dot_nt(v_.pop(("o", hh)), _ld(wot[hh]))
                v_["acc"] = d if hh == 0 else v_["acc"] + d
                if hh == H - 1:
                    outv[pl.ds(r0, seg), 0:Dm] = v_["acc"][M:, :].astype(BF16)
                    st["mem"] = v_["acc"][:M, :]

            qk = [_Op("qk%d" % i, 160, [(prev, LAT_M)] if (i == 0 and prev) else [],
                      functools.partial(f_qk, i)) for i in range(H)]
            vv = [_Op("v%d" % i, 80, [], functools.partial(f_v, i)) for i in range(H)]
            ss = [_Op("s%d" % i, 20, [(qk[i], LAT_S)], functools.partial(f_s, i)) for i in range(H)]
            oo = [_Op("o%d" % i, 20, [(ss[i], LAT_O), (vv[i], LAT_S)], functools.partial(f_o, i)) for i in range(H)]
            rr = [_Op("r%d" % i, 80, [(oo[i], LAT_R)], functools.partial(f_r, i)) for i in range(H)]
            q = []
            for t in range(H + 3):
                if t < H:
                    q.append(qk[t])
                if 0 <= t - 1 < H:
                    q.append(ss[t - 1])
                    q.append(vv[t - 1])
                if 0 <= t - 2 < H:
                    q.append(oo[t - 2])
                if 0 <= t - 3 < H:
                    q.append(rr[t - 3])
            return q

        def b_ops(h):
            v_ = {}
            KT = KC // BQ

            def chunks(i):
                return [(t0, min(t0 + KT, i + 1)) for t0 in range(0, i + 1, KT)]

            def f_qk(i, t0, t1):
                qt = _ld(qt_all[h, :, BQ * i:BQ * (i + 1)])
                k0, k1 = BQ * t0, BQ * t1
                km = (k0 + k1) // 2
                sc = jnp.concatenate([_dot(_ld(kh[k0 // 2:km // 2, :]), qt), _dot(_ld(kh[km // 2:k1 // 2, :]), qt)], axis=0)
                if t1 == i + 1:
                    sd = jnp.where(cmask, sc[k1 - k0 - BQ:, :], NEG)
                    sc = jnp.concatenate([sc[:k1 - k0 - BQ, :], sd], axis=0) if t1 - t0 > 1 else sd
                v_["s", i, t0] = sc
                m = jnp.max(sc.reshape((k1 - k0) // RM, RM, BQ), axis=0)
                v_["m", i] = m if t0 == 0 else jnp.maximum(v_["m", i], m)
                if t1 == i + 1:
                    v_["m", i] = jnp.max(v_["m", i], axis=0, keepdims=True)

            def f_e(i, t0, t1, e0, e1):
                p = jnp.exp2(v_["s", i, t0][e0:e1, :] - v_["m", i])
                l = jnp.sum(p.reshape((e1 - e0) // RS, RS, BQ), axis=0)
                v_["l", i] = l if (t0 == 0 and e0 == 0) else v_["l", i] + l
                v_.setdefault(("p", i, t0), []).append(p.astype(BF16))

            def f_pv(i, t0, t1):
                p = jnp.concatenate(v_.pop(("p", i, t0)), axis=0)
                ns = {0: 1, 1: 4, 2: 2, 3: 4}[(t1 - t0) % 4]
                rr = Dh // ns
                d = jnp.concatenate([_dot(_ld(vth[r * rr // 2:(r + 1) * rr // 2, BQ * t0:BQ * t1]), p) for r in range(ns)], axis=0)
                v_["c", i] = d if t0 == 0 else v_["c", i] + d
                if t1 == i + 1:
                    r = 1.0 / jnp.sum(v_.pop(("l", i)), axis=0, keepdims=True)
                    v_["c", i] = (v_["c", i] * r).astype(BF16)

            def f_op(i):
                ct = v_.pop(("c", i))
                hm = Dm // 2
                for r in range(2):
                    acct[PAD + r * hm:PAD + (r + 1) * hm, BQ * i:BQ * (i + 1)] += _dot(
                        _ld(bwot[h, r * hm // 2:(r + 1) * hm // 2, :]), ct)

            P = functools.partial
            qk = [[_Op("QK%d" % i, 64 * (t1 - t0), [], P(f_qk, i, t0, t1)) for t0, t1 in chunks(i)]
                  for i in range(nqb)]
            epv = []
            for i in range(nqb):
                es = [[_Op("E", 0, [(qk[i][-1], LAT_BP)], P(f_e, i, t0, t1, e0, min(e0 + EC, BQ * (t1 - t0))))
                       for e0 in range(0, BQ * (t1 - t0), EC)] for t0, t1 in chunks(i)]
                pv = [_Op("PV%d" % i, 64 * (t1 - t0), [(es[n][-1], LAT_BE)], P(f_pv, i, t0, t1))
                      for n, (t0, t1) in enumerate(chunks(i))]
                l = list(es[0])
                for n in range(len(pv)):
                    if n + 1 < len(pv):
                        l += es[n + 1]
                    l.append(pv[n])
                epv.append(l)
            op = [_Op("OP%d" % i, 224, [(epv[i][-1], LAT_BO)], P(f_op, i)) for i in range(nqb)]
            q = []
            order = ORDER(nqb)
            for t in range(nqb + 2):
                l1 = qk[order[t]] if t < nqb else []
                l2 = epv[order[t - 1]] if 0 <= t - 1 < nqb else []
                keyed = [((n + 0.25) / len(l1), 0, o) for n, o in enumerate(l1)]
                keyed += [((n + 0.75) / len(l2), 1, o) for n, o in enumerate(l2)]
                q += [o for _, _, o in sorted(keyed, key=lambda z: z[:2])]
                if 0 <= t - 2 < nqb:
                    q.append(op[order[t - 2]])
            return q

        def head(h, carry):
            if DO_B:
                shift = (16 * (1 - h % 2)).astype(U32)
                with jax.named_scope('s_kv'):
                    def kvb(n, carry):
                        r0 = pl.multiple_of(n * KVC, KVC)
                        r2 = pl.multiple_of(n * (KVC // 2), KVC // 2)
                        kh[pl.ds(r2, KVC // 2), :] = _pk(
                            _dot(_ld(c[pl.ds(r2, KVC // 2), :]), _unpack(ruk[h // 2], shift)))
                        vth[:, pl.ds(r0, KVC)] = _pk(
                            _dot_nt(_unpack(ruv[h // 2].T, shift), _ld(c[pl.ds(r2, KVC // 2), :])))
                        return carry
                    lax.fori_loop(0, S // KVC, kvb, 0)

            @pl.when((h % 2 == 0) & (h < H - 2))
            def _():
                for cp in kv_copies(h // 2 + 1):
                    cp.start()

            @pl.when((h % 2 == 1) & (h < H - 1))
            def _():
                for cp in kv_copies(h // 2 + 1):
                    cp.wait()

            st = {"mem": memf[...]}
            qa = []
            if DO_A:
                for t in range(seg_per_head):
                    qa += a_ops(h * seg_per_head + t, st, qa[-1] if qa else None)
            qb = b_ops(h) if DO_B else []
            with jax.named_scope('s_att'):
                for o in _merge(qa, qb):
                    o.fn()
            memf[...] = st["mem"]
            return carry

        with jax.named_scope('s_heads'):
            lax.fori_loop(0, H, head, 0)

        lane = lax.broadcasted_iota(jnp.int32, (OB, 128), 1)
        cps = []
        for r in range(S // OB):
            bt = acct[:, OB * r:OB * (r + 1)].T.astype(BF16)
            rows = slice(OB * r, OB * (r + 1))
            outv[rows, LO:LO + 128] = jnp.where(lane < 128 - PAD, outv[rows, LO:LO + 128], bt[:, 0:128])
            outv[rows, LO + 128:] = bt[:, 128:]
            cp = pltpu.make_async_copy(outv.at[rows], out_hbm.at[rows], sems.at[7, r])
            cp.start()
            cps.append(cp)
        for cp in cps:
            cp.wait()

    return kernel


@functools.partial(jax.jit, static_argnames=("A_seg_len",))
def pallas_concat_heads__memory_aug_recurrent_mem_tr__compressed_kv_cla__prompt_kernel(A_x, A_mem0, A_Wq, A_Wk, A_Wv, A_Wo, A_seg_len, B_x, B_c_kv, B_w_q, B_w_uk, B_w_uv, B_w_o):
    _, S, Dm = A_x.shape
    M = A_mem0.shape[1]
    H, Dh = A_Wq.shape[1], A_Wq.shape[2]
    Dc = B_c_kv.shape[2]
    seg = int(A_seg_len)
    kern = _make_kernel(S, Dm, H, Dh, M, seg, Dc)
    any_spec = pl.BlockSpec(memory_space=pl.ANY)
    scratch = [
        pltpu.VMEM((Dm, S), BF16),
        pltpu.VMEM((S // 2, Dm), U32),
        pltpu.VMEM((M, Dm), BF16),
        pltpu.VMEM((H // 2, Dm, Dh), U32),
        pltpu.VMEM((H // 2, Dm, Dh), U32),
        pltpu.VMEM((H // 2, Dm, Dh), U32),
        pltpu.VMEM((Dm // 2, 3 * H * Dh), U32),
        pltpu.VMEM((H, Dm // 2, Dh), U32),
        pltpu.VMEM((Dm // 2, S), U32),
        pltpu.VMEM((S // 2, Dc), U32),
        pltpu.VMEM((H // 2, Dm, Dh), U32),
        pltpu.VMEM((H // 2, Dc, Dh), U32),
        pltpu.VMEM((H // 2, Dc, Dh), U32),
        pltpu.VMEM((H, Dm // 2, Dh), U32),
        pltpu.VMEM((H, Dh // 2, S), U32),
        pltpu.VMEM((M, Dm), F32),
        pltpu.VMEM((S // 2, Dh), U32),
        pltpu.VMEM((Dh // 2, S), U32),
        pltpu.VMEM((Dm + (-Dm) % 128, S), F32),
        pltpu.VMEM((S, 2 * Dm), BF16),
        pltpu.SemaphoreType.DMA((11, 8)),
    ]
    out = pl.pallas_call(
        kern,
        out_shape=jax.ShapeDtypeStruct((S, 2 * Dm), BF16),
        in_specs=[any_spec] * 12,
        out_specs=any_spec,
        scratch_shapes=scratch,
        compiler_params=pltpu.CompilerParams(vmem_limit_bytes=120 * 1024 * 1024),
    )(A_x[0].T, A_mem0.reshape(M, Dm), A_Wq, A_Wk, A_Wv, jnp.swapaxes(A_Wo, 1, 2),
      B_x[0].T, B_c_kv.reshape(S, Dc), B_w_q, B_w_uk, B_w_uv, jnp.swapaxes(B_w_o, 1, 2))
    return out.reshape(1, S, 2 * Dm)
```

```python
import functools
import jax
import jax.numpy as jnp
import numpy as np
from jax import lax
from jax.experimental import pallas as pl
from jax.experimental.pallas import tpu as pltpu

F32 = jnp.float32
BF16 = jnp.bfloat16
U32 = jnp.uint32
NEG = -1000000000.0

DO_A = True
DO_B = True
LAT_S = 250
LAT_O = 250
LAT_R = 120
LAT_M = 150
LAT_BP = 300
LAT_BO = 150
VERBOSE = False
LOG2E = 1.4426950408889634
OB = 256
BIAS = 0.04
KC = 256
RM = 32
RS = 16
KVC = 1024
EC = 128
LAT_BE = 150
ORDER = lambda n: list(range(n - 1, -1, -1))


def _dot(a, b):
    return lax.dot_general(a, b, (((1,), (0,)), ((), ())), preferred_element_type=F32)


def _dot_nt(a, b):
    return lax.dot_general(a, b, (((1,), (1,)), ((), ())), preferred_element_type=F32)


def _unpack(u, shift):
    w = (u << shift) & jnp.uint32(0xFFFF0000)
    return pltpu.bitcast(w, F32).astype(BF16)


def _ld(words):
    return pltpu.bitcast(words, BF16)


def _pk(x):
    return pltpu.bitcast(x.astype(BF16), U32)


class _Op:
    def __init__(self, name, cost, deps, fn):
        self.name, self.cost, self.deps, self.fn = name, cost, deps, fn
        self.end = None


def _merge(qa, qb):
    ta = sum(o.cost for o in qa) or 1
    tb = sum(o.cost for o in qb) or 1
    ia = ib = 0
    da = db = 0
    t = 0
    order = []
    stall = 0

    def ready(o):
        return max([0] + [d.end + lat for d, lat in o.deps])

    while ia < len(qa) or ib < len(qb):
        cand = []
        if ia < len(qa):
            cand.append((max(ready(qa[ia]), t), da / ta, 0))
        if ib < len(qb):
            cand.append((max(ready(qb[ib]), t), db / tb + BIAS, 1))
        st, _, w = min(cand)
        o = qa[ia] if w == 0 else qb[ib]
        stall += st - t
        t = st + o.cost
        o.end = t
        order.append(o)
        if w == 0:
            ia += 1
            da += o.cost
        else:
            ib += 1
            db += o.cost
    if VERBOSE:
        print("sim total", t, "stall", stall)
        print(" ".join(o.name for o in order))
    return order


def _make_kernel(S, Dm, H, Dh, M, seg, Dc):
    n_seg = S // seg
    seg_per_head = n_seg // H
    L = M + seg
    BQ = 128
    nqb = S // BQ
    scale = Dh ** (-0.5) * LOG2E
    PAD = (-Dm) % 128
    LO = Dm + PAD - 128

    def kernel(xat_hbm, mem0_hbm, wq_hbm, wk_hbm, wv_hbm, wot_hbm,
               xbt_hbm, c_hbm, bwq_hbm, wuk_hbm, wuv_hbm, bwot_hbm,
               out_hbm,
               xat, xa, mem0, rq, rk, rv, wqkv, wot,
               xbt, c, rbq, ruk, ruv, bwot,
               qt_all, wqt, memf, kh, vth, acct, outv, sems):

        NP = H // 2

        def pcopy(src, dst, j, s0):
            return pltpu.make_async_copy(src.bitcast(U32).at[:, j, :], dst.at[j], sems.at[s0, j])

        def q_copies(j):
            return [pcopy(bwq_hbm, rbq, j, 0)]

        def a_copies(j):
            return [pcopy(wq_hbm, rq, j, 1), pcopy(wk_hbm, rk, j, 2), pcopy(wv_hbm, rv, j, 3)]

        def kv_copies(j):
            return [pcopy(wuk_hbm, ruk, j, 4), pcopy(wuv_hbm, ruv, j, 5)]

        cp_x = pltpu.make_async_copy(xbt_hbm.bitcast(U32), xbt, sems.at[6, 0])
        cp_xa = pltpu.make_async_copy(xat_hbm, xat, sems.at[6, 1])
        cp_m = pltpu.make_async_copy(mem0_hbm, mem0, sems.at[6, 3])
        NL = NP // 2
        CR = S // NL // 2
        HL = H // NL

        def rest_copies(j):
            r0 = pl.multiple_of(j * CR, CR)
            return [pltpu.make_async_copy(c_hbm.bitcast(U32).at[pl.ds(r0, CR)], c.at[pl.ds(r0, CR)], sems.at[8, j]),
                    pltpu.make_async_copy(wot_hbm.bitcast(U32).at[pl.ds(HL * j, HL)], wot.at[pl.ds(HL * j, HL)],
                                          sems.at[9, j]),
                    pltpu.make_async_copy(bwot_hbm.bitcast(U32).at[pl.ds(HL * j, HL)], bwot.at[pl.ds(HL * j, HL)],
                                          sems.at[10, j])]

        for cp in q_copies(0) + [cp_x] + q_copies(1):
            cp.start()

        def zero(r, carry):
            acct[:, pl.ds(pl.multiple_of(r * 128, 128), 128)] = jnp.zeros((acct.shape[0], 128), F32)
            return carry

        lax.fori_loop(0, S // 128, zero, 0)

        def q_weights(j):
            ut = rbq[j].T
            for par in range(2):
                wqt[j % 2, par] = _pk(_unpack(ut, 16 * (1 - par)))

        with jax.named_scope('s_q0wait'):
            for cp in q_copies(0):
                cp.wait()
        q_weights(0)
        with jax.named_scope('s_xwait'):
            cp_x.wait()
        cp_xa.start()
        cp_m.start()

        def q_pair(j, fill):
            nchunk = 8
            cw = S // nchunk
            slots = 2 * nchunk - 1
            for par in range(2):
                for n in range(nchunk):
                    qt_all[2 * j + par, :, n * cw:(n + 1) * cw] = _pk(
                        _dot(_ld(wqt[j % 2, par]), _ld(xbt[:, n * cw:(n + 1) * cw])) * scale)
                    u = par * nchunk + n
                    for f in fill[len(fill) * u // slots:len(fill) * (u + 1) // slots]:
                        f()

        def qproj1(j, carry):
            for cp in q_copies(j + 2) + a_copies(2 * j) + a_copies(2 * j + 1):
                cp.start()
            for cp in q_copies(j + 1):
                cp.wait()
            q_pair(j, [functools.partial(q_weights, j + 1)])
            return carry

        def qproj2(jj, carry):
            j = jj + NL
            for cp in rest_copies(jj):
                cp.start()

            @pl.when(j + 2 < NP)
            def _():
                for cp in q_copies(j + 2):
                    cp.start()

            @pl.when(j + 2 == NP)
            def _():
                for cp in kv_copies(0):
                    cp.start()

            @pl.when(j + 1 < NP)
            def _():
                for cp in q_copies(j + 1):
                    cp.wait()

            for cp in a_copies(2 * jj) + a_copies(2 * jj + 1):
                cp.wait()

            def a_unpack(ja, wi, par):
                c0 = pl.multiple_of(wi * H * Dh + (2 * ja + par) * Dh, Dh)
                wqkv[:, pl.ds(c0, Dh)] = _pk(_unpack((rq, rk, rv)[wi][ja], 16 * (1 - par)))

            def tr(u):
                n = S // NP
                r0 = pl.multiple_of((2 * jj + u) * n, n)
                xa[pl.ds(pl.multiple_of((2 * jj + u) * (n // 2), n // 2), n // 2), :] = _pk(xat[:, pl.ds(r0, n)].T)

            def next_weights():
                jn = jnp.minimum(j + 1, NP - 1)
                ut = rbq[jn].T
                for par in range(2):
                    wqt[(j + 1) % 2, par] = _pk(_unpack(ut, 16 * (1 - par)))

            fill = [next_weights, functools.partial(tr, 0), functools.partial(tr, 1)]
            fill += [functools.partial(a_unpack, 2 * jj + d, wi, par)
                     for d in range(2) for wi in range(3) for par in range(2)]
            q_pair(j, fill)
            return carry

        with jax.named_scope('s_qproj'):
            lax.fori_loop(0, NL, qproj1, 0)
            cp_xa.wait()
            lax.fori_loop(0, NL, qproj2, 0)

        with jax.named_scope('s_wait2'):
            for j in range(NL):
                for cp in rest_copies(j):
                    cp.wait()
            for cp in kv_copies(0) + [cp_m]:
                cp.wait()

        RH = seg_per_head * seg

        def early_out(h):
            r0 = h * RH if isinstance(h, int) else pl.multiple_of(h * RH, RH)
            return pltpu.make_async_copy(outv.at[pl.ds(r0, RH), pl.ds(0, LO)],
                                         out_hbm.at[pl.ds(r0, RH), pl.ds(0, LO)], sems.at[11 + h // 8, h % 8])

        memf[...] = mem0[...].astype(F32)
        krow = lax.broadcasted_iota(jnp.int32, (BQ, BQ), 0)
        qcol = lax.broadcasted_iota(jnp.int32, (BQ, BQ), 1)
        cmask = krow <= qcol
        arow = lax.broadcasted_iota(jnp.int32, (L, L), 0)
        acol = lax.broadcasted_iota(jnp.int32, (L, L), 1)
        amask = (arow < M) | (arow >= acol)

        def a_ops(s, st, prev):
            r0 = pl.multiple_of(s * seg, seg)
            v_ = {}

            def f_qk(hh):
                if hh == 0:
                    xs = _ld(xa[pl.ds(pl.multiple_of(s * (seg // 2), seg // 2), seg // 2), :]).astype(F32)
                    v_["h"] = jnp.concatenate([st["mem"], xs], axis=0)
                hc = v_["h"]
                v_["q", hh] = _dot(hc, _ld(wqkv[:, hh * Dh:(hh + 1) * Dh])) * scale
                v_["k", hh] = _dot(hc, _ld(wqkv[:, (H + hh) * Dh:(H + hh + 1) * Dh])).astype(BF16)

            def f_v(hh):
                v_["v", hh] = _dot(v_["h"], _ld(wqkv[:, (2 * H + hh) * Dh:(2 * H + hh + 1) * Dh])).astype(BF16)

            def f_s(hh):
                sc = _dot_nt(v_.pop(("q", hh)), v_.pop(("k", hh)))
                sc = jnp.where(amask, sc, NEG)
                m = jnp.max(sc, axis=-1, keepdims=True)
                p = jnp.exp2(sc - m)
                v_["p", hh] = p
                v_["r", hh] = 1.0 / jnp.sum(p, axis=-1, keepdims=True)

            def f_o(hh):
                v_["o", hh] = _dot(v_.pop(("p", hh)), v_.pop(("v", hh))) * v_.pop(("r", hh))

            def f_r(hh):
                d = _dot_nt(v_.pop(("o", hh)), _ld(wot[hh]))
                v_["acc"] = d if hh == 0 else v_["acc"] + d
                if hh == H - 1:
                    outv[pl.ds(r0, seg), 0:Dm] = v_["acc"][M:, :].astype(BF16)
                    st["mem"] = v_["acc"][:M, :]

            qk = [_Op("qk%d" % i, 160, [(prev, LAT_M)] if (i == 0 and prev) else [],
                      functools.partial(f_qk, i)) for i in range(H)]
            vv = [_Op("v%d" % i, 80, [], functools.partial(f_v, i)) for i in range(H)]
            ss = [_Op("s%d" % i, 20, [(qk[i], LAT_S)], functools.partial(f_s, i)) for i in range(H)]
            oo = [_Op("o%d" % i, 20, [(ss[i], LAT_O), (vv[i], LAT_S)], functools.partial(f_o, i)) for i in range(H)]
            rr = [_Op("r%d" % i, 80, [(oo[i], LAT_R)], functools.partial(f_r, i)) for i in range(H)]
            q = []
            for t in range(H + 3):
                if t < H:
                    q.append(qk[t])
                if 0 <= t - 1 < H:
                    q.append(ss[t - 1])
                    q.append(vv[t - 1])
                if 0 <= t - 2 < H:
                    q.append(oo[t - 2])
                if 0 <= t - 3 < H:
                    q.append(rr[t - 3])
            return q

        def b_ops(h):
            v_ = {}
            KT = KC // BQ

            def chunks(i):
                return [(t0, min(t0 + KT, i + 1)) for t0 in range(0, i + 1, KT)]

            def f_qk(i, t0, t1):
                qt = _ld(qt_all[h, :, BQ * i:BQ * (i + 1)])
                k0, k1 = BQ * t0, BQ * t1
                km = (k0 + k1) // 2
                sc = jnp.concatenate([_dot(_ld(kh[k0 // 2:km // 2, :]), qt), _dot(_ld(kh[km // 2:k1 // 2, :]), qt)], axis=0)
                if t1 == i + 1:
                    sd = jnp.where(cmask, sc[k1 - k0 - BQ:, :], NEG)
                    sc = jnp.concatenate([sc[:k1 - k0 - BQ, :], sd], axis=0) if t1 - t0 > 1 else sd
                v_["s", i, t0] = sc
                m = jnp.max(sc.reshape((k1 - k0) // RM, RM, BQ), axis=0)
                v_["m", i] = m if t0 == 0 else jnp.maximum(v_["m", i], m)
                if t1 == i + 1:
                    v_["m", i] = jnp.max(v_["m", i], axis=0, keepdims=True)

            def f_e(i, t0, t1, e0, e1):
                p = jnp.exp2(v_["s", i, t0][e0:e1, :] - v_["m", i])
                l = jnp.sum(p.reshape((e1 - e0) // RS, RS, BQ), axis=0)
                v_["l", i] = l if (t0 == 0 and e0 == 0) else v_["l", i] + l
                v_.setdefault(("p", i, t0), []).append(p.astype(BF16))

            def f_pv(i, t0, t1):
                p = jnp.concatenate(v_.pop(("p", i, t0)), axis=0)
                ns = {0: 1, 1: 4, 2: 2, 3: 4}[(t1 - t0) % 4]
                rr = Dh // ns
                d = jnp.concatenate([_dot(_ld(vth[r * rr // 2:(r + 1) * rr // 2, BQ * t0:BQ * t1]), p) for r in range(ns)], axis=0)
                v_["c", i] = d if t0 == 0 else v_["c", i] + d
                if t1 == i + 1:
                    r = 1.0 / jnp.sum(v_.pop(("l", i)), axis=0, keepdims=True)
                    v_["c", i] = (v_["c", i] * r).astype(BF16)

            def f_op(i):
                ct = v_.pop(("c", i))
                hm = Dm // 2
                for r in range(2):
                    acct[PAD + r * hm:PAD + (r + 1) * hm, BQ * i:BQ * (i + 1)] += _dot(
                        _ld(bwot[h, r * hm // 2:(r + 1) * hm // 2, :]), ct)

            P = functools.partial
            qk = [[_Op("QK%d" % i, 64 * (t1 - t0), [], P(f_qk, i, t0, t1)) for t0, t1 in chunks(i)]
                  for i in range(nqb)]
            epv = []
            for i in range(nqb):
                es = [[_Op("E", 0, [(qk[i][-1], LAT_BP)], P(f_e, i, t0, t1, e0, min(e0 + EC, BQ * (t1 - t0))))
                       for e0 in range(0, BQ * (t1 - t0), EC)] for t0, t1 in chunks(i)]
                pv = [_Op("PV%d" % i, 64 * (t1 - t0), [(es[n][-1], LAT_BE)], P(f_pv, i, t0, t1))
                      for n, (t0, t1) in enumerate(chunks(i))]
                l = list(es[0])
                for n in range(len(pv)):
                    if n + 1 < len(pv):
                        l += es[n + 1]
                    l.append(pv[n])
                epv.append(l)
            op = [_Op("OP%d" % i, 224, [(epv[i][-1], LAT_BO)], P(f_op, i)) for i in range(nqb)]
            q = []
            order = ORDER(nqb)
            for t in range(nqb + 2):
                l1 = qk[order[t]] if t < nqb else []
                l2 = epv[order[t - 1]] if 0 <= t - 1 < nqb else []
                keyed = [((n + 0.25) / len(l1), 0, o) for n, o in enumerate(l1)]
                keyed += [((n + 0.75) / len(l2), 1, o) for n, o in enumerate(l2)]
                q += [o for _, _, o in sorted(keyed, key=lambda z: z[:2])]
                if 0 <= t - 2 < nqb:
                    q.append(op[order[t - 2]])
            return q

        def head(h, carry):
            if DO_B:
                shift = (16 * (1 - h % 2)).astype(U32)
                with jax.named_scope('s_kv'):
                    def kvb(n, carry):
                        r0 = pl.multiple_of(n * KVC, KVC)
                        r2 = pl.multiple_of(n * (KVC // 2), KVC // 2)
                        kh[pl.ds(r2, KVC // 2), :] = _pk(
                            _dot(_ld(c[pl.ds(r2, KVC // 2), :]), _unpack(ruk[h // 2], shift)))
                        vth[:, pl.ds(r0, KVC)] = _pk(
                            _dot_nt(_unpack(ruv[h // 2].T, shift), _ld(c[pl.ds(r2, KVC // 2), :])))
                        return carry
                    lax.fori_loop(0, S // KVC, kvb, 0)

            @pl.when((h % 2 == 0) & (h < H - 2))
            def _():
                for cp in kv_copies(h // 2 + 1):
                    cp.start()

            @pl.when((h % 2 == 1) & (h < H - 1))
            def _():
                for cp in kv_copies(h // 2 + 1):
                    cp.wait()

            @pl.when(h > 0)
            def _():
                early_out(h - 1).start()

            st = {"mem": memf[...]}
            qa = []
            if DO_A:
                for t in range(seg_per_head):
                    qa += a_ops(h * seg_per_head + t, st, qa[-1] if qa else None)
            qb = b_ops(h) if DO_B else []
            with jax.named_scope('s_att'):
                for o in _merge(qa, qb):
                    o.fn()
            memf[...] = st["mem"]
            return carry

        with jax.named_scope('s_heads'):
            lax.fori_loop(0, H, head, 0)

        def out_copy(r):
            r0 = pl.multiple_of(r * OB, OB)
            return pltpu.make_async_copy(outv.at[pl.ds(r0, OB), pl.ds(LO, 2 * Dm - LO)],
                                         out_hbm.at[pl.ds(r0, OB), pl.ds(LO, 2 * Dm - LO)], sems.at[7, r])

        def epi(r, carry):
            lane = lax.broadcasted_iota(jnp.int32, (OB, 128), 1)
            rows = pl.ds(pl.multiple_of(r * OB, OB), OB)
            bt = acct[:, rows].T.astype(BF16)
            outv[rows, LO:LO + 128] = jnp.where(lane < 128 - PAD, outv[rows, LO:LO + 128], bt[:, 0:128])
            outv[rows, LO + 128:] = bt[:, 128:]
            out_copy(r).start()
            return carry

        with jax.named_scope('s_epi'):
            early_out(H - 1).start()
            lax.fori_loop(0, S // OB, epi, 0)
            for hh in range(H):
                early_out(hh).wait()
            for r in range(S // OB):
                out_copy(r).wait()

    return kernel


@functools.partial(jax.jit, static_argnames=("A_seg_len",))
def pallas_concat_heads__memory_aug_recurrent_mem_tr__compressed_kv_cla__prompt_kernel(A_x, A_mem0, A_Wq, A_Wk, A_Wv, A_Wo, A_seg_len, B_x, B_c_kv, B_w_q, B_w_uk, B_w_uv, B_w_o):
    _, S, Dm = A_x.shape
    M = A_mem0.shape[1]
    H, Dh = A_Wq.shape[1], A_Wq.shape[2]
    Dc = B_c_kv.shape[2]
    seg = int(A_seg_len)
    kern = _make_kernel(S, Dm, H, Dh, M, seg, Dc)
    any_spec = pl.BlockSpec(memory_space=pl.ANY)
    scratch = [
        pltpu.VMEM((Dm, S), BF16),
        pltpu.VMEM((S // 2, Dm), U32),
        pltpu.VMEM((M, Dm), BF16),
        pltpu.VMEM((H // 2, Dm, Dh), U32),
        pltpu.VMEM((H // 2, Dm, Dh), U32),
        pltpu.VMEM((H // 2, Dm, Dh), U32),
        pltpu.VMEM((Dm // 2, 3 * H * Dh), U32),
        pltpu.VMEM((H, Dm // 2, Dh), U32),
        pltpu.VMEM((Dm // 2, S), U32),
        pltpu.VMEM((S // 2, Dc), U32),
        pltpu.VMEM((H // 2, Dm, Dh), U32),
        pltpu.VMEM((H // 2, Dc, Dh), U32),
        pltpu.VMEM((H // 2, Dc, Dh), U32),
        pltpu.VMEM((H, Dm // 2, Dh), U32),
        pltpu.VMEM((H, Dh // 2, S), U32),
        pltpu.VMEM((2, 2, Dh // 2, Dm), U32),
        pltpu.VMEM((M, Dm), F32),
        pltpu.VMEM((S // 2, Dh), U32),
        pltpu.VMEM((Dh // 2, S), U32),
        pltpu.VMEM((Dm + (-Dm) % 128, S), F32),
        pltpu.VMEM((S, 2 * Dm), BF16),
        pltpu.SemaphoreType.DMA((13, 8)),
    ]
    out = pl.pallas_call(
        kern,
        out_shape=jax.ShapeDtypeStruct((S, 2 * Dm), BF16),
        in_specs=[any_spec] * 12,
        out_specs=any_spec,
        scratch_shapes=scratch,
        compiler_params=pltpu.CompilerParams(vmem_limit_bytes=120 * 1024 * 1024),
    )(A_x[0].T, A_mem0.reshape(M, Dm), A_Wq, A_Wk, A_Wv, jnp.swapaxes(A_Wo, 1, 2),
      B_x[0].T, B_c_kv.reshape(S, Dc), B_w_q, B_w_uk, B_w_uv, jnp.swapaxes(B_w_o, 1, 2))
    return out.reshape(1, S, 2 * Dm)
```

```python
import functools
import jax
import jax.numpy as jnp
import numpy as np
from jax import lax
from jax.experimental import pallas as pl
from jax.experimental.pallas import tpu as pltpu

F32 = jnp.float32
BF16 = jnp.bfloat16
U32 = jnp.uint32
NEG = -1000000000.0

DO_A = True
DO_B = True
LAT_S = 250
LAT_O = 250
LAT_R = 120
LAT_M = 150
LAT_BP = 300
LAT_BO = 150
VERBOSE = False
LOG2E = 1.4426950408889634
OB = 256
BIAS = 0.04
KC = 256
RM = 32
RS = 16
KVC = 1024
KM = 128
EC = 128
LAT_BE = 150
ORDER = lambda n: list(range(n - 1, -1, -1))


def _dot(a, b):
    return lax.dot_general(a, b, (((1,), (0,)), ((), ())), preferred_element_type=F32)


def _dot_nt(a, b):
    return lax.dot_general(a, b, (((1,), (1,)), ((), ())), preferred_element_type=F32)


def _unpack(u, shift):
    w = (u << shift) & jnp.uint32(0xFFFF0000)
    return pltpu.bitcast(w, F32).astype(BF16)


def _unpack_f32(u, shift):
    return pltpu.bitcast((u << shift) & jnp.uint32(0xFFFF0000), F32)


def _ld(words):
    return pltpu.bitcast(words, BF16)


def _pk(x):
    return pltpu.bitcast(x.astype(BF16), U32)


class _Op:
    def __init__(self, name, cost, deps, fn):
        self.name, self.cost, self.deps, self.fn = name, cost, deps, fn
        self.end = None


def _merge(qa, qb):
    ta = sum(o.cost for o in qa) or 1
    tb = sum(o.cost for o in qb) or 1
    ia = ib = 0
    da = db = 0
    t = 0
    order = []
    stall = 0

    def ready(o):
        return max([0] + [d.end + lat for d, lat in o.deps])

    while ia < len(qa) or ib < len(qb):
        cand = []
        if ia < len(qa):
            cand.append((max(ready(qa[ia]), t), da / ta, 0))
        if ib < len(qb):
            cand.append((max(ready(qb[ib]), t), db / tb + BIAS, 1))
        st, _, w = min(cand)
        o = qa[ia] if w == 0 else qb[ib]
        stall += st - t
        t = st + o.cost
        o.end = t
        order.append(o)
        if w == 0:
            ia += 1
            da += o.cost
        else:
            ib += 1
            db += o.cost
    if VERBOSE:
        print("sim total", t, "stall", stall)
        print(" ".join(o.name for o in order))
    return order


def _make_kernel(S, Dm, H, Dh, M, seg, Dc):
    n_seg = S // seg
    seg_per_head = n_seg // H
    L = M + seg
    BQ = 128
    nqb = S // BQ
    scale = Dh ** (-0.5) * LOG2E
    PAD = (-Dm) % 128
    LO = Dm + PAD - 128

    def kernel(xat_hbm, mem0_hbm, wq_hbm, wk_hbm, wv_hbm, wot_hbm,
               xbt_hbm, c_hbm, bwq_hbm, wuk_hbm, wuv_hbm, bwot_hbm,
               out_hbm,
               xat, xa, mem0, rq, rk, rv, wqkv, wot,
               xbt, c, rbq, ruk, ruv, bwot,
               qt_all, cs, wqt, memf, kh, vth, acct, outv, sems):

        NP = H // 2

        def pcopy(src, dst, j, s0):
            return pltpu.make_async_copy(src.bitcast(U32).at[:, j, :], dst.at[j], sems.at[s0, j])

        def q_copies(j):
            return [pcopy(bwq_hbm, rbq, j, 0)]

        def a_copies(j):
            return [pcopy(wq_hbm, rq, j, 1), pcopy(wk_hbm, rk, j, 2), pcopy(wv_hbm, rv, j, 3)]

        def kv_copies(j):
            return [pcopy(wuk_hbm, ruk, j, 4), pcopy(wuv_hbm, ruv, j, 5)]

        cp_x = pltpu.make_async_copy(xbt_hbm.bitcast(U32), xbt, sems.at[6, 0])
        cp_xa = pltpu.make_async_copy(xat_hbm, xat, sems.at[6, 1])
        cp_m = pltpu.make_async_copy(mem0_hbm, mem0, sems.at[6, 3])
        NL = NP // 2
        CR = S // NL // 2
        HL = H // NL

        def rest_copies(j):
            r0 = pl.multiple_of(j * CR, CR)
            return [pltpu.make_async_copy(c_hbm.bitcast(U32).at[pl.ds(r0, CR)], c.at[pl.ds(r0, CR)], sems.at[8, j]),
                    pltpu.make_async_copy(wot_hbm.bitcast(U32).at[pl.ds(HL * j, HL)], wot.at[pl.ds(HL * j, HL)],
                                          sems.at[9, j]),
                    pltpu.make_async_copy(bwot_hbm.bitcast(U32).at[pl.ds(HL * j, HL)], bwot.at[pl.ds(HL * j, HL)],
                                          sems.at[10, j])]

        for cp in q_copies(0) + [cp_x] + q_copies(1):
            cp.start()

        def zero(r, carry):
            acct[:, pl.ds(pl.multiple_of(r * 128, 128), 128)] = jnp.zeros((acct.shape[0], 128), F32)
            return carry

        lax.fori_loop(0, S // 128, zero, 0)

        def q_weights(j):
            ut = rbq[j].T
            for par in range(2):
                wqt[j % 2, par] = _pk(_unpack(ut, 16 * (1 - par)))

        with jax.named_scope('s_q0wait'):
            for cp in q_copies(0):
                cp.wait()
        q_weights(0)
        with jax.named_scope('s_xwait'):
            cp_x.wait()
        cp_xa.start()
        cp_m.start()

        def q_pair(j, fill):
            nchunk = 8
            cw = S // nchunk
            slots = 2 * nchunk - 1
            for par in range(2):
                for n in range(nchunk):
                    qt_all[2 * j + par, :, n * cw:(n + 1) * cw] = _pk(
                        _dot(_ld(wqt[j % 2, par]), _ld(xbt[:, n * cw:(n + 1) * cw])) * scale)
                    u = par * nchunk + n
                    for f in fill[len(fill) * u // slots:len(fill) * (u + 1) // slots]:
                        f()

        def qproj1(j, carry):
            for cp in q_copies(j + 2) + a_copies(2 * j) + a_copies(2 * j + 1):
                cp.start()
            for cp in q_copies(j + 1):
                cp.wait()
            q_pair(j, [functools.partial(q_weights, j + 1)])
            return carry

        def qproj2(jj, carry):
            j = jj + NL
            for cp in rest_copies(jj):
                cp.start()

            @pl.when(j + 2 < NP)
            def _():
                for cp in q_copies(j + 2):
                    cp.start()

            @pl.when(j + 2 == NP)
            def _():
                for cp in kv_copies(0):
                    cp.start()

            @pl.when(j + 1 < NP)
            def _():
                for cp in q_copies(j + 1):
                    cp.wait()

            for cp in a_copies(2 * jj) + a_copies(2 * jj + 1):
                cp.wait()

            def a_unpack(ja, wi, par):
                c0 = pl.multiple_of(wi * H * Dh + (2 * ja + par) * Dh, Dh)
                wqkv[:, pl.ds(c0, Dh)] = _pk(_unpack((rq, rk, rv)[wi][ja], 16 * (1 - par)))

            def tr(u):
                n = S // NP
                r0 = pl.multiple_of((2 * jj + u) * n, n)
                xa[pl.ds(pl.multiple_of((2 * jj + u) * (n // 2), n // 2), n // 2), :] = _pk(xat[:, pl.ds(r0, n)].T)

            def next_weights():
                jn = jnp.minimum(j + 1, NP - 1)
                ut = rbq[jn].T
                for par in range(2):
                    wqt[(j + 1) % 2, par] = _pk(_unpack(ut, 16 * (1 - par)))

            fill = [next_weights, functools.partial(tr, 0), functools.partial(tr, 1)]
            fill += [functools.partial(a_unpack, 2 * jj + d, wi, par)
                     for d in range(2) for wi in range(3) for par in range(2)]
            q_pair(j, fill)
            return carry

        with jax.named_scope('s_qproj'):
            lax.fori_loop(0, NL, qproj1, 0)
            cp_xa.wait()
            lax.fori_loop(0, NL, qproj2, 0)

        with jax.named_scope('s_wait2'):
            for j in range(NL):
                for cp in rest_copies(j):
                    cp.wait()
            for cp in kv_copies(0) + [cp_m]:
                cp.wait()

        KH = KVC // 2
        DH2 = Dc // 2

        def csum(t, carry):
            n, r = t // (KH // 128), t % (KH // 128)
            top = pl.ds(pl.multiple_of(n * (KVC // 2) + r * 64, 64), 64)
            bot = pl.ds(pl.multiple_of(n * (KVC // 2) + KH // 2 + r * 64, 64), 64)
            a11, a12 = _ld(c[top, 0:DH2]).astype(F32), _ld(c[top, DH2:]).astype(F32)
            a21, a22 = _ld(c[bot, 0:DH2]).astype(F32), _ld(c[bot, DH2:]).astype(F32)
            dst = pl.ds(pl.multiple_of(t * 64, 64), 64)
            for i, x in enumerate((a11 + a22, a21 + a22, a11 + a12, a21 - a11, a12 - a22)):
                cs[i, dst, :] = _pk(x)
            return carry

        lax.fori_loop(0, S // 256, csum, 0)

        RH = seg_per_head * seg

        def early_out(h):
            r0 = h * RH if isinstance(h, int) else pl.multiple_of(h * RH, RH)
            return pltpu.make_async_copy(outv.at[pl.ds(r0, RH), pl.ds(0, LO)],
                                         out_hbm.at[pl.ds(r0, RH), pl.ds(0, LO)], sems.at[11 + h // 8, h % 8])

        memf[...] = mem0[...].astype(F32)
        krow = lax.broadcasted_iota(jnp.int32, (BQ, BQ), 0)
        qcol = lax.broadcasted_iota(jnp.int32, (BQ, BQ), 1)
        cmask = krow <= qcol
        arow = lax.broadcasted_iota(jnp.int32, (L, L), 0)
        acol = lax.broadcasted_iota(jnp.int32, (L, L), 1)
        amask = (arow < M) | (arow >= acol)

        def a_ops(s, st, prev):
            r0 = pl.multiple_of(s * seg, seg)
            v_ = {}

            def f_qk(hh):
                if hh == 0:
                    xs = _ld(xa[pl.ds(pl.multiple_of(s * (seg // 2), seg // 2), seg // 2), :]).astype(F32)
                    v_["h"] = jnp.concatenate([st["mem"], xs], axis=0)
                hc = v_["h"]
                v_["q", hh] = _dot(hc, _ld(wqkv[:, hh * Dh:(hh + 1) * Dh])) * scale
                v_["k", hh] = _dot(hc, _ld(wqkv[:, (H + hh) * Dh:(H + hh + 1) * Dh])).astype(BF16)

            def f_v(hh):
                v_["v", hh] = _dot(v_["h"], _ld(wqkv[:, (2 * H + hh) * Dh:(2 * H + hh + 1) * Dh])).astype(BF16)

            def f_s(hh):
                sc = _dot_nt(v_.pop(("q", hh)), v_.pop(("k", hh)))
                sc = jnp.where(amask, sc, NEG)
                m = jnp.max(sc, axis=-1, keepdims=True)
                p = jnp.exp2(sc - m)
                v_["p", hh] = p
                v_["r", hh] = 1.0 / jnp.sum(p, axis=-1, keepdims=True)

            def f_o(hh):
                v_["o", hh] = _dot(v_.pop(("p", hh)), v_.pop(("v", hh))) * v_.pop(("r", hh))

            def f_r(hh):
                d = _dot_nt(v_.pop(("o", hh)), _ld(wot[hh]))
                v_["acc"] = d if hh == 0 else v_["acc"] + d
                if hh == H - 1:
                    outv[pl.ds(r0, seg), 0:Dm] = v_["acc"][M:, :].astype(BF16)
                    st["mem"] = v_["acc"][:M, :]

            qk = [_Op("qk%d" % i, 160, [(prev, LAT_M)] if (i == 0 and prev) else [],
                      functools.partial(f_qk, i)) for i in range(H)]
            vv = [_Op("v%d" % i, 80, [], functools.partial(f_v, i)) for i in range(H)]
            ss = [_Op("s%d" % i, 20, [(qk[i], LAT_S)], functools.partial(f_s, i)) for i in range(H)]
            oo = [_Op("o%d" % i, 20, [(ss[i], LAT_O), (vv[i], LAT_S)], functools.partial(f_o, i)) for i in range(H)]
            rr = [_Op("r%d" % i, 80, [(oo[i], LAT_R)], functools.partial(f_r, i)) for i in range(H)]
            q = []
            for t in range(H + 3):
                if t < H:
                    q.append(qk[t])
                if 0 <= t - 1 < H:
                    q.append(ss[t - 1])
                    q.append(vv[t - 1])
                if 0 <= t - 2 < H:
                    q.append(oo[t - 2])
                if 0 <= t - 3 < H:
                    q.append(rr[t - 3])
            return q

        def b_ops(h):
            v_ = {}
            KT = KC // BQ

            def chunks(i):
                return [(t0, min(t0 + KT, i + 1)) for t0 in range(0, i + 1, KT)]

            def f_qk(i, t0, t1):
                qt = _ld(qt_all[h, :, BQ * i:BQ * (i + 1)])
                k0, k1 = BQ * t0, BQ * t1
                km = (k0 + k1) // 2
                sc = jnp.concatenate([_dot(_ld(kh[k0 // 2:km // 2, :]), qt), _dot(_ld(kh[km // 2:k1 // 2, :]), qt)], axis=0)
                if t1 == i + 1:
                    sd = jnp.where(cmask, sc[k1 - k0 - BQ:, :], NEG)
                    sc = jnp.concatenate([sc[:k1 - k0 - BQ, :], sd], axis=0) if t1 - t0 > 1 else sd
                v_["s", i, t0] = sc
                m = jnp.max(sc.reshape((k1 - k0) // RM, RM, BQ), axis=0)
                v_["m", i] = m if t0 == 0 else jnp.maximum(v_["m", i], m)
                if t1 == i + 1:
                    v_["m", i] = jnp.max(v_["m", i], axis=0, keepdims=True)

            def f_e(i, t0, t1, e0, e1):
                p = jnp.exp2(v_["s", i, t0][e0:e1, :] - v_["m", i])
                l = jnp.sum(p.reshape((e1 - e0) // RS, RS, BQ), axis=0)
                v_["l", i] = l if (t0 == 0 and e0 == 0) else v_["l", i] + l
                v_.setdefault(("p", i, t0), []).append(p.astype(BF16))

            def f_pv(i, t0, t1):
                p = jnp.concatenate(v_.pop(("p", i, t0)), axis=0)
                ns = {0: 1, 1: 4, 2: 2, 3: 4}[(t1 - t0) % 4]
                rr = Dh // ns
                d = jnp.concatenate([_dot(_ld(vth[r * rr // 2:(r + 1) * rr // 2, BQ * t0:BQ * t1]), p) for r in range(ns)], axis=0)
                v_["c", i] = d if t0 == 0 else v_["c", i] + d
                if t1 == i + 1:
                    r = 1.0 / jnp.sum(v_.pop(("l", i)), axis=0, keepdims=True)
                    v_["c", i] = (v_["c", i] * r).astype(BF16)

            def f_op(i):
                ct = v_.pop(("c", i))
                hm = Dm // 2
                for r in range(2):
                    acct[PAD + r * hm:PAD + (r + 1) * hm, BQ * i:BQ * (i + 1)] += _dot(
                        _ld(bwot[h, r * hm // 2:(r + 1) * hm // 2, :]), ct)

            P = functools.partial
            qk = [[_Op("QK%d" % i, 64 * (t1 - t0), [], P(f_qk, i, t0, t1)) for t0, t1 in chunks(i)]
                  for i in range(nqb)]
            epv = []
            for i in range(nqb):
                es = [[_Op("E", 0, [(qk[i][-1], LAT_BP)], P(f_e, i, t0, t1, e0, min(e0 + EC, BQ * (t1 - t0))))
                       for e0 in range(0, BQ * (t1 - t0), EC)] for t0, t1 in chunks(i)]
                pv = [_Op("PV%d" % i, 64 * (t1 - t0), [(es[n][-1], LAT_BE)], P(f_pv, i, t0, t1))
                      for n, (t0, t1) in enumerate(chunks(i))]
                l = list(es[0])
                for n in range(len(pv)):
                    if n + 1 < len(pv):
                        l += es[n + 1]
                    l.append(pv[n])
                epv.append(l)
            op = [_Op("OP%d" % i, 224, [(epv[i][-1], LAT_BO)], P(f_op, i)) for i in range(nqb)]
            q = []
            order = ORDER(nqb)
            for t in range(nqb + 2):
                l1 = qk[order[t]] if t < nqb else []
                l2 = epv[order[t - 1]] if 0 <= t - 1 < nqb else []
                keyed = [((n + 0.25) / len(l1), 0, o) for n, o in enumerate(l1)]
                keyed += [((n + 0.75) / len(l2), 1, o) for n, o in enumerate(l2)]
                q += [o for _, _, o in sorted(keyed, key=lambda z: z[:2])]
                if 0 <= t - 2 < nqb:
                    q.append(op[order[t - 2]])
            return q

        def head(h, carry):
            if DO_B:
                shift = (16 * (1 - h % 2)).astype(U32)
                with jax.named_scope('s_kv'):
                    def kvb(n, carry):
                        def wcombos(w11, w12, w21, w22):
                            f = lambda x: x.astype(BF16)
                            return [f(w11 + w22), f(w11), f(w12 - w22), f(w21 - w11), f(w22), f(w11 + w12),
                                    f(w21 + w22)]

                        def lhs(p, r, m):
                            if p == 2:
                                return _ld(c[pl.ds(pl.multiple_of(n * (KVC // 2) + r // 2, 8), m // 2), 0:DH2])
                            if p == 3:
                                return _ld(c[pl.ds(pl.multiple_of(n * (KVC // 2) + (KH + r) // 2, 8), m // 2), DH2:])
                            return _ld(cs[(0, 1, None, None, 2, 3, 4)[p],
                                          pl.ds(pl.multiple_of(n * (KH // 2) + r // 2, 8), m // 2), :])

                        def outs(m):
                            return (m[0] + m[3] - m[4] + m[6], m[2] + m[4], m[1] + m[3], m[0] - m[1] + m[2] + m[5])

                        wk = _unpack_f32(ruk[h // 2], shift)
                        wc = wcombos(wk[:DH2, :128], wk[:DH2, 128:], wk[DH2:, :128], wk[DH2:, 128:])
                        for r in range(0, KH, KM):
                            c11, c12, c21, c22 = outs([_dot(lhs(p, r, KM), wc[p]) for p in range(7)])
                            top = pl.ds(pl.multiple_of(n * (KVC // 2) + r // 2, 8), KM // 2)
                            bot = pl.ds(pl.multiple_of(n * (KVC // 2) + (KH + r) // 2, 8), KM // 2)
                            kh[top, 0:128] = _pk(c11)
                            kh[top, 128:] = _pk(c12)
                            kh[bot, 0:128] = _pk(c21)
                            kh[bot, 128:] = _pk(c22)
                        wv = _unpack_f32(ruv[h // 2].T, shift)
                        wc = wcombos(wv[:128, :DH2], wv[128:, :DH2], wv[:128, DH2:], wv[128:, DH2:])
                        for r in range(0, KH, 128):
                            c11, c12, c21, c22 = outs([_dot_nt(wc[p], lhs(p, r, 128)) for p in range(7)])
                            top = pl.ds(pl.multiple_of(n * KVC + r, 128), 128)
                            bot = pl.ds(pl.multiple_of(n * KVC + KH + r, 128), 128)
                            vth[0:64, top] = _pk(c11)
                            vth[64:, top] = _pk(c12)
                            vth[0:64, bot] = _pk(c21)
                            vth[64:, bot] = _pk(c22)
                        return carry
                    lax.fori_loop(0, S // KVC, kvb, 0)

            @pl.when((h % 2 == 0) & (h < H - 2))
            def _():
                for cp in kv_copies(h // 2 + 1):
                    cp.start()

            @pl.when((h % 2 == 1) & (h < H - 1))
            def _():
                for cp in kv_copies(h // 2 + 1):
                    cp.wait()

            @pl.when(h > 0)
            def _():
                early_out(h - 1).start()

            st = {"mem": memf[...]}
            qa = []
            if DO_A:
                for t in range(seg_per_head):
                    qa += a_ops(h * seg_per_head + t, st, qa[-1] if qa else None)
            qb = b_ops(h) if DO_B else []
            with jax.named_scope('s_att'):
                for o in _merge(qa, qb):
                    o.fn()
            memf[...] = st["mem"]
            return carry

        with jax.named_scope('s_heads'):
            lax.fori_loop(0, H, head, 0)

        def out_copy(r):
            r0 = pl.multiple_of(r * OB, OB)
            return pltpu.make_async_copy(outv.at[pl.ds(r0, OB), pl.ds(LO, 2 * Dm - LO)],
                                         out_hbm.at[pl.ds(r0, OB), pl.ds(LO, 2 * Dm - LO)], sems.at[7, r])

        def epi(r, carry):
            lane = lax.broadcasted_iota(jnp.int32, (OB, 128), 1)
            rows = pl.ds(pl.multiple_of(r * OB, OB), OB)
            bt = acct[:, rows].T.astype(BF16)
            outv[rows, LO:LO + 128] = jnp.where(lane < 128 - PAD, outv[rows, LO:LO + 128], bt[:, 0:128])
            outv[rows, LO + 128:] = bt[:, 128:]
            out_copy(r).start()
            return carry

        with jax.named_scope('s_epi'):
            early_out(H - 1).start()
            lax.fori_loop(0, S // OB, epi, 0)
            for hh in range(H):
                early_out(hh).wait()
            for r in range(S // OB):
                out_copy(r).wait()

    return kernel


@functools.partial(jax.jit, static_argnames=("A_seg_len",))
def pallas_concat_heads__memory_aug_recurrent_mem_tr__compressed_kv_cla__prompt_kernel(A_x, A_mem0, A_Wq, A_Wk, A_Wv, A_Wo, A_seg_len, B_x, B_c_kv, B_w_q, B_w_uk, B_w_uv, B_w_o):
    _, S, Dm = A_x.shape
    M = A_mem0.shape[1]
    H, Dh = A_Wq.shape[1], A_Wq.shape[2]
    Dc = B_c_kv.shape[2]
    seg = int(A_seg_len)
    kern = _make_kernel(S, Dm, H, Dh, M, seg, Dc)
    any_spec = pl.BlockSpec(memory_space=pl.ANY)
    scratch = [
        pltpu.VMEM((Dm, S), BF16),
        pltpu.VMEM((S // 2, Dm), U32),
        pltpu.VMEM((M, Dm), BF16),
        pltpu.VMEM((H // 2, Dm, Dh), U32),
        pltpu.VMEM((H // 2, Dm, Dh), U32),
        pltpu.VMEM((H // 2, Dm, Dh), U32),
        pltpu.VMEM((Dm // 2, 3 * H * Dh), U32),
        pltpu.VMEM((H, Dm // 2, Dh), U32),
        pltpu.VMEM((Dm // 2, S), U32),
        pltpu.VMEM((S // 2, Dc), U32),
        pltpu.VMEM((H // 2, Dm, Dh), U32),
        pltpu.VMEM((H // 2, Dc, Dh), U32),
        pltpu.VMEM((H // 2, Dc, Dh), U32),
        pltpu.VMEM((H, Dm // 2, Dh), U32),
        pltpu.VMEM((H, Dh // 2, S), U32),
        pltpu.VMEM((5, S // 4, Dc // 2), U32),
        pltpu.VMEM((2, 2, Dh // 2, Dm), U32),
        pltpu.VMEM((M, Dm), F32),
        pltpu.VMEM((S // 2, Dh), U32),
        pltpu.VMEM((Dh // 2, S), U32),
        pltpu.VMEM((Dm + (-Dm) % 128, S), F32),
        pltpu.VMEM((S, 2 * Dm), BF16),
        pltpu.SemaphoreType.DMA((13, 8)),
    ]
    out = pl.pallas_call(
        kern,
        out_shape=jax.ShapeDtypeStruct((S, 2 * Dm), BF16),
        in_specs=[any_spec] * 12,
        out_specs=any_spec,
        scratch_shapes=scratch,
        compiler_params=pltpu.CompilerParams(vmem_limit_bytes=120 * 1024 * 1024),
    )(A_x[0].T, A_mem0.reshape(M, Dm), A_Wq, A_Wk, A_Wv, jnp.swapaxes(A_Wo, 1, 2),
      B_x[0].T, B_c_kv.reshape(S, Dc), B_w_q, B_w_uk, B_w_uv, jnp.swapaxes(B_w_o, 1, 2))
    return out.reshape(1, S, 2 * Dm)
```

```python
import functools
import jax
import jax.numpy as jnp
import numpy as np
from jax import lax
from jax.experimental import pallas as pl
from jax.experimental.pallas import tpu as pltpu

F32 = jnp.float32
BF16 = jnp.bfloat16
U32 = jnp.uint32
NEG = -1000000000.0

DO_A = True
DO_B = True
LAT_S = 250
LAT_O = 250
LAT_R = 120
LAT_M = 150
LAT_BP = 300
LAT_BO = 150
VERBOSE = False
LOG2E = 1.4426950408889634
OB = 256
BIAS = 0.04
KC = 256
RM = 32
RS = 16
KVC = 1024
KM = 128
EC = 128
LAT_BE = 150
ORDER = lambda n: list(range(n - 1, -1, -1))


def _dot(a, b):
    return lax.dot_general(a, b, (((1,), (0,)), ((), ())), preferred_element_type=F32)


def _dot_nt(a, b):
    return lax.dot_general(a, b, (((1,), (1,)), ((), ())), preferred_element_type=F32)


def _unpack(u, shift):
    w = (u << shift) & jnp.uint32(0xFFFF0000)
    return pltpu.bitcast(w, F32).astype(BF16)


def _unpack_f32(u, shift):
    return pltpu.bitcast((u << shift) & jnp.uint32(0xFFFF0000), F32)


def _ld(words):
    return pltpu.bitcast(words, BF16)


def _pk(x):
    return pltpu.bitcast(x.astype(BF16), U32)


class _Op:
    def __init__(self, name, cost, deps, fn):
        self.name, self.cost, self.deps, self.fn = name, cost, deps, fn
        self.end = None


def _merge(qa, qb):
    ta = sum(o.cost for o in qa) or 1
    tb = sum(o.cost for o in qb) or 1
    ia = ib = 0
    da = db = 0
    t = 0
    order = []
    stall = 0

    def ready(o):
        return max([0] + [d.end + lat for d, lat in o.deps])

    while ia < len(qa) or ib < len(qb):
        cand = []
        if ia < len(qa):
            cand.append((max(ready(qa[ia]), t), da / ta, 0))
        if ib < len(qb):
            cand.append((max(ready(qb[ib]), t), db / tb + BIAS, 1))
        st, _, w = min(cand)
        o = qa[ia] if w == 0 else qb[ib]
        stall += st - t
        t = st + o.cost
        o.end = t
        order.append(o)
        if w == 0:
            ia += 1
            da += o.cost
        else:
            ib += 1
            db += o.cost
    if VERBOSE:
        print("sim total", t, "stall", stall)
        print(" ".join(o.name for o in order))
    return order


def _make_kernel(S, Dm, H, Dh, M, seg, Dc):
    n_seg = S // seg
    seg_per_head = n_seg // H
    L = M + seg
    BQ = 128
    nqb = S // BQ
    scale = Dh ** (-0.5) * LOG2E
    PAD = (-Dm) % 128
    LO = Dm + PAD - 128

    def kernel(xat_hbm, mem0_hbm, wq_hbm, wk_hbm, wv_hbm, wot_hbm,
               xbt_hbm, c_hbm, bwq_hbm, wuk_hbm, wuv_hbm, bwot_hbm,
               out_hbm,
               xat, xa, mem0, rq, rk, rv, wqk, wvo, wot,
               xbt, c, rbq, ruk, ruv, bwot,
               qt_all, cs, wqt, memf, kh, vth, acct, outv, sems):

        NP = H // 2

        def pcopy(src, dst, j, s0):
            return pltpu.make_async_copy(src.bitcast(U32).at[:, j, :], dst.at[j], sems.at[s0, j])

        def q_copies(j):
            return [pcopy(bwq_hbm, rbq, j, 0)]

        def a_copies(j):
            return [pcopy(wq_hbm, rq, j, 1), pcopy(wk_hbm, rk, j, 2), pcopy(wv_hbm, rv, j, 3),
                    pltpu.make_async_copy(wot_hbm.bitcast(U32).at[pl.ds(2 * j, 2)], wot.at[pl.ds(2 * j, 2)],
                                          sems.at[9, j])]

        def kv_copies(j):
            return [pcopy(wuk_hbm, ruk, j, 4), pcopy(wuv_hbm, ruv, j, 5)]

        cp_x = pltpu.make_async_copy(xbt_hbm.bitcast(U32), xbt, sems.at[6, 0])
        cp_xa = pltpu.make_async_copy(xat_hbm, xat, sems.at[6, 1])
        cp_m = pltpu.make_async_copy(mem0_hbm, mem0, sems.at[6, 3])
        NL = NP // 2
        CR = S // NL // 2
        HL = H // NL

        def rest_copies(j):
            r0 = pl.multiple_of(j * CR, CR)
            return [pltpu.make_async_copy(c_hbm.bitcast(U32).at[pl.ds(r0, CR)], c.at[pl.ds(r0, CR)], sems.at[8, j]),
                    pltpu.make_async_copy(bwot_hbm.bitcast(U32).at[pl.ds(HL * j, HL)], bwot.at[pl.ds(HL * j, HL)],
                                          sems.at[10, j])]

        for cp in q_copies(0) + [cp_x] + q_copies(1):
            cp.start()

        def zero(r, carry):
            acct[:, pl.ds(pl.multiple_of(r * 128, 128), 128)] = jnp.zeros((acct.shape[0], 128), F32)
            return carry

        lax.fori_loop(0, S // 128, zero, 0)

        def q_weights(j):
            ut = rbq[j].T
            for par in range(2):
                wqt[j % 2, par] = _pk(_unpack(ut, 16 * (1 - par)))

        with jax.named_scope('s_q0wait'):
            for cp in q_copies(0):
                cp.wait()
        q_weights(0)
        with jax.named_scope('s_xwait'):
            cp_x.wait()
        cp_xa.start()
        cp_m.start()

        def q_pair(j, fill):
            nchunk = 8
            cw = S // nchunk
            slots = 2 * nchunk - 1
            for par in range(2):
                for n in range(nchunk):
                    qt_all[2 * j + par, :, n * cw:(n + 1) * cw] = _pk(
                        _dot(_ld(wqt[j % 2, par]), _ld(xbt[:, n * cw:(n + 1) * cw])) * scale)
                    u = par * nchunk + n
                    for f in fill[len(fill) * u // slots:len(fill) * (u + 1) // slots]:
                        f()

        def qproj1(j, carry):
            for cp in q_copies(j + 2) + a_copies(2 * j) + a_copies(2 * j + 1):
                cp.start()
            for cp in q_copies(j + 1):
                cp.wait()
            q_pair(j, [functools.partial(q_weights, j + 1)])
            return carry

        def qproj2(jj, carry):
            j = jj + NL
            for cp in rest_copies(jj):
                cp.start()

            @pl.when(j + 2 < NP)
            def _():
                for cp in q_copies(j + 2):
                    cp.start()

            @pl.when(j + 2 == NP)
            def _():
                for cp in kv_copies(0):
                    cp.start()

            @pl.when(j + 1 < NP)
            def _():
                for cp in q_copies(j + 1):
                    cp.wait()

            for cp in a_copies(2 * jj) + a_copies(2 * jj + 1):
                cp.wait()

            def a_unpack(ja, wi, par):
                c0 = pl.multiple_of(wi * H * Dh + (2 * ja + par) * Dh, Dh)
                wqk[:, pl.ds(c0, Dh)] = _pk(_unpack((rq, rk)[wi][ja], 16 * (1 - par)))

            def a_vo(ja):
                zero = jnp.zeros((PAD // 2, Dh), U32)
                ev = _dot_nt(_unpack(rv[ja], 16), _ld(jnp.concatenate([wot[2 * ja], zero], axis=0)))
                od = _dot_nt(_unpack(rv[ja], 0), _ld(jnp.concatenate([zero, wot[2 * ja + 1]], axis=0)))
                wvo[ja, :, 0:LO] = _pk(ev[:, :LO])
                wvo[ja, :, LO:LO + 128] = _pk(ev[:, LO:] + od[:, :128])
                wvo[ja, :, LO + 128:] = _pk(od[:, 128:])

            def tr(u):
                n = S // NP
                r0 = pl.multiple_of((2 * jj + u) * n, n)
                xa[pl.ds(pl.multiple_of((2 * jj + u) * (n // 2), n // 2), n // 2), :] = _pk(xat[:, pl.ds(r0, n)].T)

            def next_weights():
                jn = jnp.minimum(j + 1, NP - 1)
                ut = rbq[jn].T
                for par in range(2):
                    wqt[(j + 1) % 2, par] = _pk(_unpack(ut, 16 * (1 - par)))

            fill = [next_weights, functools.partial(tr, 0), functools.partial(tr, 1)]
            for d in range(2):
                fill += [functools.partial(a_unpack, 2 * jj + d, wi, par) for wi in range(2) for par in range(2)]
                fill += [functools.partial(a_vo, 2 * jj + d)]
            q_pair(j, fill)
            return carry

        with jax.named_scope('s_qproj'):
            lax.fori_loop(0, NL, qproj1, 0)
            cp_xa.wait()
            lax.fori_loop(0, NL, qproj2, 0)

        with jax.named_scope('s_wait2'):
            for j in range(NL):
                for cp in rest_copies(j):
                    cp.wait()
            for cp in kv_copies(0) + [cp_m]:
                cp.wait()

        KH = KVC // 2
        DH2 = Dc // 2

        def csum(t, carry):
            n, r = t // (KH // 128), t % (KH // 128)
            top = pl.ds(pl.multiple_of(n * (KVC // 2) + r * 64, 64), 64)
            bot = pl.ds(pl.multiple_of(n * (KVC // 2) + KH // 2 + r * 64, 64), 64)
            a11, a12 = _ld(c[top, 0:DH2]).astype(F32), _ld(c[top, DH2:]).astype(F32)
            a21, a22 = _ld(c[bot, 0:DH2]).astype(F32), _ld(c[bot, DH2:]).astype(F32)
            dst = pl.ds(pl.multiple_of(t * 64, 64), 64)
            for i, x in enumerate((a11 + a22, a21 + a22, a11 + a12, a21 - a11, a12 - a22)):
                cs[i, dst, :] = _pk(x)
            return carry

        lax.fori_loop(0, S // 256, csum, 0)

        RH = seg_per_head * seg

        def early_out(h):
            r0 = h * RH if isinstance(h, int) else pl.multiple_of(h * RH, RH)
            return pltpu.make_async_copy(outv.at[pl.ds(r0, RH), pl.ds(0, LO)],
                                         out_hbm.at[pl.ds(r0, RH), pl.ds(0, LO)], sems.at[11 + h // 8, h % 8])

        memf[...] = mem0[...].astype(F32)
        krow = lax.broadcasted_iota(jnp.int32, (BQ, BQ), 0)
        qcol = lax.broadcasted_iota(jnp.int32, (BQ, BQ), 1)
        cmask = krow <= qcol
        GH = 128 // L
        arow = lax.broadcasted_iota(jnp.int32, (L, 128), 0)
        alane = lax.broadcasted_iota(jnp.int32, (L, 128), 1)
        aseg = sum((alane >= L * i).astype(jnp.int32) for i in range(1, GH + 1))
        acol = alane - L * aseg
        amask = (arow < M) | (arow >= acol)
        NPAIR = H // 2
        groups = [list(range(g, min(g + GH, NPAIR))) for g in range(0, NPAIR, GH)]
        UW = 2 * Dm

        def a_ops(s, st, prev):
            r0 = pl.multiple_of(s * seg, seg)
            v_ = {}

            def f_qk(hh):
                if hh == 0:
                    xs = _ld(xa[pl.ds(pl.multiple_of(s * (seg // 2), seg // 2), seg // 2), :]).astype(F32)
                    v_["h"] = jnp.concatenate([st["mem"], xs], axis=0)
                hc = v_["h"]
                v_["q", hh] = _dot(hc, _ld(wqk[:, hh * Dh:(hh + 1) * Dh])) * scale
                v_["k", hh] = _dot(hc, _ld(wqk[:, (H + hh) * Dh:(H + hh + 1) * Dh]))

            def f_u(j):
                v_["u", j] = _dot(v_["h"], _ld(wvo[j]))

            def rows_at(parts):
                used = sum(p.shape[0] for p in parts)
                pad = [jnp.zeros((128 - used, parts[0].shape[1]), F32)]
                return jnp.concatenate(parts + pad, axis=0).astype(BF16)

            def f_s(g, par):
                sc = None
                for i, j in enumerate(groups[g]):
                    hh = 2 * j + par
                    lead = [jnp.zeros((L * i, Dh), F32)] if i else []
                    d = _dot_nt(v_.pop(("q", hh)), rows_at(lead + [v_.pop(("k", hh))]))
                    sc = d if sc is None else sc + d
                n = len(groups[g])
                sc = jnp.where(amask & (aseg < n), sc, NEG)
                m = None
                for i in range(n):
                    mi = jnp.max(jnp.where(aseg == i, sc, -jnp.inf), axis=-1, keepdims=True)
                    m = mi if m is None else jnp.where(aseg == i, mi, m)
                p = jnp.where(aseg < n, jnp.exp2(sc - m), 0.0)
                l = None
                for i in range(n):
                    li = jnp.sum(jnp.where(aseg == i, p, 0.0), axis=-1, keepdims=True)
                    l = li if l is None else jnp.where(aseg == i, li, l)
                v_["p", g, par] = p / l

            def f_o(g, par):
                c0 = par * LO
                d = _dot(v_.pop(("p", g, par)), rows_at([v_["u", j][:, c0:c0 + Dm + PAD] for j in groups[g]]))
                v_["acc", par] = d if g == 0 else v_["acc", par] + d
                if g == len(groups) - 1 and par == 1:
                    o = v_["acc", 0][:, :Dm] + v_["acc", 1][:, PAD:]
                    outv[pl.ds(r0, seg), 0:Dm] = o[M:, :].astype(BF16)
                    st["mem"] = o[:M, :]

            P = functools.partial
            qk = [_Op("qk%d" % i, 160, [(prev, LAT_M)] if (i == 0 and prev) else [], P(f_qk, i)) for i in range(H)]
            uu = [_Op("u%d" % j, 280, [], P(f_u, j)) for j in range(NPAIR)]
            q = []
            pend = []
            for g, prs in enumerate(groups):
                for hh in range(2 * prs[0], 2 * prs[-1] + 2):
                    q.append(qk[hh])
                    if pend:
                        q.append(pend.pop(0))
                q.append(uu[prs[0]])
                ss = [_Op("s", 20 * len(prs), [(qk[2 * prs[-1] + par], LAT_S)], P(f_s, g, par)) for par in range(2)]
                q += ss
                q += [uu[j] for j in prs[1:]]
                pend = [_Op("o", 40, [(ss[par], LAT_O), (uu[prs[-1]], LAT_R)], P(f_o, g, par)) for par in range(2)]
            return q + pend

        def b_ops(h):
            v_ = {}
            KT = KC // BQ

            def chunks(i):
                return [(t0, min(t0 + KT, i + 1)) for t0 in range(0, i + 1, KT)]

            def f_qk(i, t0, t1):
                qt = _ld(qt_all[h, :, BQ * i:BQ * (i + 1)])
                k0, k1 = BQ * t0, BQ * t1
                km = (k0 + k1) // 2
                sc = jnp.concatenate([_dot(_ld(kh[k0 // 2:km // 2, :]), qt), _dot(_ld(kh[km // 2:k1 // 2, :]), qt)], axis=0)
                if t1 == i + 1:
                    sd = jnp.where(cmask, sc[k1 - k0 - BQ:, :], NEG)
                    sc = jnp.concatenate([sc[:k1 - k0 - BQ, :], sd], axis=0) if t1 - t0 > 1 else sd
                v_["s", i, t0] = sc
                m = jnp.max(sc.reshape((k1 - k0) // RM, RM, BQ), axis=0)
                v_["m", i] = m if t0 == 0 else jnp.maximum(v_["m", i], m)
                if t1 == i + 1:
                    v_["m", i] = jnp.max(v_["m", i], axis=0, keepdims=True)

            def f_e(i, t0, t1, e0, e1):
                p = jnp.exp2(v_["s", i, t0][e0:e1, :] - v_["m", i])
                l = jnp.sum(p.reshape((e1 - e0) // RS, RS, BQ), axis=0)
                v_["l", i] = l if (t0 == 0 and e0 == 0) else v_["l", i] + l
                v_.setdefault(("p", i, t0), []).append(p.astype(BF16))

            def f_pv(i, t0, t1):
                p = jnp.concatenate(v_.pop(("p", i, t0)), axis=0)
                ns = {0: 1, 1: 4, 2: 2, 3: 4}[(t1 - t0) % 4]
                rr = Dh // ns
                d = jnp.concatenate([_dot(_ld(vth[r * rr // 2:(r + 1) * rr // 2, BQ * t0:BQ * t1]), p) for r in range(ns)], axis=0)
                v_["c", i] = d if t0 == 0 else v_["c", i] + d
                if t1 == i + 1:
                    r = 1.0 / jnp.sum(v_.pop(("l", i)), axis=0, keepdims=True)
                    v_["c", i] = (v_["c", i] * r).astype(BF16)

            def f_op(i):
                ct = v_.pop(("c", i))
                hm = Dm // 2
                for r in range(2):
                    acct[PAD + r * hm:PAD + (r + 1) * hm, BQ * i:BQ * (i + 1)] += _dot(
                        _ld(bwot[h, r * hm // 2:(r + 1) * hm // 2, :]), ct)

            P = functools.partial
            qk = [[_Op("QK%d" % i, 64 * (t1 - t0), [], P(f_qk, i, t0, t1)) for t0, t1 in chunks(i)]
                  for i in range(nqb)]
            epv = []
            for i in range(nqb):
                es = [[_Op("E", 0, [(qk[i][-1], LAT_BP)], P(f_e, i, t0, t1, e0, min(e0 + EC, BQ * (t1 - t0))))
                       for e0 in range(0, BQ * (t1 - t0), EC)] for t0, t1 in chunks(i)]
                pv = [_Op("PV%d" % i, 64 * (t1 - t0), [(es[n][-1], LAT_BE)], P(f_pv, i, t0, t1))
                      for n, (t0, t1) in enumerate(chunks(i))]
                l = list(es[0])
                for n in range(len(pv)):
                    if n + 1 < len(pv):
                        l += es[n + 1]
                    l.append(pv[n])
                epv.append(l)
            op = [_Op("OP%d" % i, 224, [(epv[i][-1], LAT_BO)], P(f_op, i)) for i in range(nqb)]
            q = []
            order = ORDER(nqb)
            for t in range(nqb + 2):
                l1 = qk[order[t]] if t < nqb else []
                l2 = epv[order[t - 1]] if 0 <= t - 1 < nqb else []
                keyed = [((n + 0.25) / len(l1), 0, o) for n, o in enumerate(l1)]
                keyed += [((n + 0.75) / len(l2), 1, o) for n, o in enumerate(l2)]
                q += [o for _, _, o in sorted(keyed, key=lambda z: z[:2])]
                if 0 <= t - 2 < nqb:
                    q.append(op[order[t - 2]])
            return q

        def head(h, carry):
            if DO_B:
                shift = (16 * (1 - h % 2)).astype(U32)
                with jax.named_scope('s_kv'):
                    def kvb(n, carry):
                        def wcombos(w11, w12, w21, w22):
                            f = lambda x: x.astype(BF16)
                            return [f(w11 + w22), f(w11), f(w12 - w22), f(w21 - w11), f(w22), f(w11 + w12),
                                    f(w21 + w22)]

                        def lhs(p, r, m):
                            if p == 2:
                                return _ld(c[pl.ds(pl.multiple_of(n * (KVC // 2) + r // 2, 8), m // 2), 0:DH2])
                            if p == 3:
                                return _ld(c[pl.ds(pl.multiple_of(n * (KVC // 2) + (KH + r) // 2, 8), m // 2), DH2:])
                            return _ld(cs[(0, 1, None, None, 2, 3, 4)[p],
                                          pl.ds(pl.multiple_of(n * (KH // 2) + r // 2, 8), m // 2), :])

                        def outs(m):
                            return (m[0] + m[3] - m[4] + m[6], m[2] + m[4], m[1] + m[3], m[0] - m[1] + m[2] + m[5])

                        wk = _unpack_f32(ruk[h // 2], shift)
                        wc = wcombos(wk[:DH2, :128], wk[:DH2, 128:], wk[DH2:, :128], wk[DH2:, 128:])
                        for r in range(0, KH, KM):
                            c11, c12, c21, c22 = outs([_dot(lhs(p, r, KM), wc[p]) for p in range(7)])
                            top = pl.ds(pl.multiple_of(n * (KVC // 2) + r // 2, 8), KM // 2)
                            bot = pl.ds(pl.multiple_of(n * (KVC // 2) + (KH + r) // 2, 8), KM // 2)
                            kh[top, 0:128] = _pk(c11)
                            kh[top, 128:] = _pk(c12)
                            kh[bot, 0:128] = _pk(c21)
                            kh[bot, 128:] = _pk(c22)
                        wv = _unpack_f32(ruv[h // 2].T, shift)
                        wc = wcombos(wv[:128, :DH2], wv[128:, :DH2], wv[:128, DH2:], wv[128:, DH2:])
                        for r in range(0, KH, 128):
                            c11, c12, c21, c22 = outs([_dot_nt(wc[p], lhs(p, r, 128)) for p in range(7)])
                            top = pl.ds(pl.multiple_of(n * KVC + r, 128), 128)
                            bot = pl.ds(pl.multiple_of(n * KVC + KH + r, 128), 128)
                            vth[0:64, top] = _pk(c11)
                            vth[64:, top] = _pk(c12)
                            vth[0:64, bot] = _pk(c21)
                            vth[64:, bot] = _pk(c22)
                        return carry
                    lax.fori_loop(0, S // KVC, kvb, 0)

            @pl.when((h % 2 == 0) & (h < H - 2))
            def _():
                for cp in kv_copies(h // 2 + 1):
                    cp.start()

            @pl.when((h % 2 == 1) & (h < H - 1))
            def _():
                for cp in kv_copies(h // 2 + 1):
                    cp.wait()

            @pl.when(h > 0)
            def _():
                early_out(h - 1).start()

            st = {"mem": memf[...]}
            qa = []
            if DO_A:
                for t in range(seg_per_head):
                    qa += a_ops(h * seg_per_head + t, st, qa[-1] if qa else None)
            qb = b_ops(h) if DO_B else []
            with jax.named_scope('s_att'):
                for o in _merge(qa, qb):
                    o.fn()
            memf[...] = st["mem"]
            return carry

        with jax.named_scope('s_heads'):
            lax.fori_loop(0, H, head, 0)

        def out_copy(r):
            r0 = pl.multiple_of(r * OB, OB)
            return pltpu.make_async_copy(outv.at[pl.ds(r0, OB), pl.ds(LO, 2 * Dm - LO)],
                                         out_hbm.at[pl.ds(r0, OB), pl.ds(LO, 2 * Dm - LO)], sems.at[7, r])

        def epi(r, carry):
            lane = lax.broadcasted_iota(jnp.int32, (OB, 128), 1)
            rows = pl.ds(pl.multiple_of(r * OB, OB), OB)
            bt = acct[:, rows].T.astype(BF16)
            outv[rows, LO:LO + 128] = jnp.where(lane < 128 - PAD, outv[rows, LO:LO + 128], bt[:, 0:128])
            outv[rows, LO + 128:] = bt[:, 128:]
            out_copy(r).start()
            return carry

        with jax.named_scope('s_epi'):
            early_out(H - 1).start()
            lax.fori_loop(0, S // OB, epi, 0)
            for hh in range(H):
                early_out(hh).wait()
            for r in range(S // OB):
                out_copy(r).wait()

    return kernel


@functools.partial(jax.jit, static_argnames=("A_seg_len",))
def pallas_concat_heads__memory_aug_recurrent_mem_tr__compressed_kv_cla__prompt_kernel(A_x, A_mem0, A_Wq, A_Wk, A_Wv, A_Wo, A_seg_len, B_x, B_c_kv, B_w_q, B_w_uk, B_w_uv, B_w_o):
    _, S, Dm = A_x.shape
    M = A_mem0.shape[1]
    H, Dh = A_Wq.shape[1], A_Wq.shape[2]
    Dc = B_c_kv.shape[2]
    seg = int(A_seg_len)
    kern = _make_kernel(S, Dm, H, Dh, M, seg, Dc)
    any_spec = pl.BlockSpec(memory_space=pl.ANY)
    scratch = [
        pltpu.VMEM((Dm, S), BF16),
        pltpu.VMEM((S // 2, Dm), U32),
        pltpu.VMEM((M, Dm), BF16),
        pltpu.VMEM((H // 2, Dm, Dh), U32),
        pltpu.VMEM((H // 2, Dm, Dh), U32),
        pltpu.VMEM((H // 2, Dm, Dh), U32),
        pltpu.VMEM((Dm // 2, 2 * H * Dh), U32),
        pltpu.VMEM((H // 2, Dm // 2, 2 * Dm), U32),
        pltpu.VMEM((H, Dm // 2, Dh), U32),
        pltpu.VMEM((Dm // 2, S), U32),
        pltpu.VMEM((S // 2, Dc), U32),
        pltpu.VMEM((H // 2, Dm, Dh), U32),
        pltpu.VMEM((H // 2, Dc, Dh), U32),
        pltpu.VMEM((H // 2, Dc, Dh), U32),
        pltpu.VMEM((H, Dm // 2, Dh), U32),
        pltpu.VMEM((H, Dh // 2, S), U32),
        pltpu.VMEM((5, S // 4, Dc // 2), U32),
        pltpu.VMEM((2, 2, Dh // 2, Dm), U32),
        pltpu.VMEM((M, Dm), F32),
        pltpu.VMEM((S // 2, Dh), U32),
        pltpu.VMEM((Dh // 2, S), U32),
        pltpu.VMEM((Dm + (-Dm) % 128, S), F32),
        pltpu.VMEM((S, 2 * Dm), BF16),
        pltpu.SemaphoreType.DMA((13, 8)),
    ]
    out = pl.pallas_call(
        kern,
        out_shape=jax.ShapeDtypeStruct((S, 2 * Dm), BF16),
        in_specs=[any_spec] * 12,
        out_specs=any_spec,
        scratch_shapes=scratch,
        compiler_params=pltpu.CompilerParams(vmem_limit_bytes=120 * 1024 * 1024),
    )(A_x[0].T, A_mem0.reshape(M, Dm), A_Wq, A_Wk, A_Wv, jnp.swapaxes(A_Wo, 1, 2),
      B_x[0].T, B_c_kv.reshape(S, Dc), B_w_q, B_w_uk, B_w_uv, jnp.swapaxes(B_w_o, 1, 2))
    return out.reshape(1, S, 2 * Dm)
```

```python
import functools
import jax
import jax.numpy as jnp
import numpy as np
from jax import lax
from jax.experimental import pallas as pl
from jax.experimental.pallas import tpu as pltpu

F32 = jnp.float32
BF16 = jnp.bfloat16
U32 = jnp.uint32
NEG = -1000000000.0

DO_A = True
DO_B = True
LAT_S = 250
LAT_O = 250
LAT_R = 120
LAT_M = 150
LAT_BP = 300
LAT_BO = 150
VERBOSE = False
LOG2E = 1.4426950408889634
OB = 256
BIAS = 0.04
KC = 256
RM = 32
RS = 16
KVC = 1024
KM = 128
KVLOOP = False
EC = 128
LAT_BE = 150
ORDER = lambda n: list(range(n - 1, -1, -1))


def _dot(a, b):
    return lax.dot_general(a, b, (((1,), (0,)), ((), ())), preferred_element_type=F32)


def _dot_nt(a, b):
    return lax.dot_general(a, b, (((1,), (1,)), ((), ())), preferred_element_type=F32)


def _unpack(u, shift):
    w = (u << shift) & jnp.uint32(0xFFFF0000)
    return pltpu.bitcast(w, F32).astype(BF16)


def _unpack_f32(u, shift):
    return pltpu.bitcast((u << shift) & jnp.uint32(0xFFFF0000), F32)


def _mo(i, n):
    return i if isinstance(i, int) else pl.multiple_of(i, n)


def _ld(words):
    return pltpu.bitcast(words, BF16)


def _pk(x):
    return pltpu.bitcast(x.astype(BF16), U32)


class _Op:
    def __init__(self, name, cost, deps, fn):
        self.name, self.cost, self.deps, self.fn = name, cost, deps, fn
        self.end = None


def _merge(qa, qb):
    ta = sum(o.cost for o in qa) or 1
    tb = sum(o.cost for o in qb) or 1
    ia = ib = 0
    da = db = 0
    t = 0
    order = []
    stall = 0

    def ready(o):
        return max([0] + [d.end + lat for d, lat in o.deps])

    while ia < len(qa) or ib < len(qb):
        cand = []
        if ia < len(qa):
            cand.append((max(ready(qa[ia]), t), da / ta, 0))
        if ib < len(qb):
            cand.append((max(ready(qb[ib]), t), db / tb + BIAS, 1))
        st, _, w = min(cand)
        o = qa[ia] if w == 0 else qb[ib]
        stall += st - t
        t = st + o.cost
        o.end = t
        order.append(o)
        if w == 0:
            ia += 1
            da += o.cost
        else:
            ib += 1
            db += o.cost
    if VERBOSE:
        print("sim total", t, "stall", stall)
        print(" ".join(o.name for o in order))
    return order


def _make_kernel(S, Dm, H, Dh, M, seg, Dc):
    n_seg = S // seg
    seg_per_head = n_seg // H
    L = M + seg
    BQ = 128
    nqb = S // BQ
    scale = Dh ** (-0.5) * LOG2E
    PAD = (-Dm) % 128
    LO = Dm + PAD - 128

    def kernel(xat_hbm, mem0_hbm, wq_hbm, wk_hbm, wv_hbm, wot_hbm,
               xbt_hbm, c_hbm, bwq_hbm, wuk_hbm, wuv_hbm, bwot_hbm,
               out_hbm,
               xat, xa, mem0, rq, rk, rv, wkq, wvo, wot,
               xbt, c, rbq, ruk, ruv, bwot,
               qt_all, cs, wqt, memf, kh, vth, acct, outv, sems):

        NP = H // 2

        def pcopy(src, dst, j, s0):
            return pltpu.make_async_copy(src.bitcast(U32).at[:, j, :], dst.at[j], sems.at[s0, j])

        def q_copies(j):
            return [pcopy(bwq_hbm, rbq, j, 0)]

        def a_copies(j):
            return [pcopy(wq_hbm, rq, j, 1), pcopy(wk_hbm, rk, j, 2), pcopy(wv_hbm, rv, j, 3),
                    pltpu.make_async_copy(wot_hbm.bitcast(U32).at[pl.ds(2 * j, 2)], wot.at[pl.ds(2 * j, 2)],
                                          sems.at[9, j])]

        def kv_copies(j):
            return [pcopy(wuk_hbm, ruk, j, 4), pcopy(wuv_hbm, ruv, j, 5)]

        cp_x = pltpu.make_async_copy(xbt_hbm.bitcast(U32), xbt, sems.at[6, 0])
        cp_xa = pltpu.make_async_copy(xat_hbm, xat, sems.at[6, 1])
        cp_m = pltpu.make_async_copy(mem0_hbm, mem0, sems.at[6, 3])
        NL = H // 2
        CR = S // NL // 2
        HL = H // NL

        def rest_copies(j):
            r0 = _mo(j * CR, CR)
            return [pltpu.make_async_copy(c_hbm.bitcast(U32).at[pl.ds(r0, CR)], c.at[pl.ds(r0, CR)], sems.at[8, j]),
                    pltpu.make_async_copy(bwot_hbm.bitcast(U32).at[pl.ds(HL * j, HL)], bwot.at[pl.ds(HL * j, HL)],
                                          sems.at[10, j])]

        for cp in q_copies(0) + [cp_x] + q_copies(1):
            cp.start()

        def zero(r, carry):
            acct[:, pl.ds(_mo(r * 128, 128), 128)] = jnp.zeros((acct.shape[0], 128), F32)
            return carry

        lax.fori_loop(0, S // 128, zero, 0)

        def q_weights(h, slot):
            wqt[slot] = _pk(_unpack(rbq[h // 2].T, (16 * (1 - h % 2)).astype(U32)))

        with jax.named_scope('s_q0wait'):
            for cp in q_copies(0):
                cp.wait()
        q_weights(jnp.int32(0), 0)
        with jax.named_scope('s_xwait'):
            cp_x.wait()
        cp_xa.start()
        cp_m.start()

        def q_head(h, fill):
            @pl.when((h % 2 == 1) & (h + 1 < H))
            def _():
                for cp in q_copies((h + 1) // 2):
                    cp.wait()

            fill = [functools.partial(q_weights, jnp.minimum(h + 1, H - 1), (h + 1) % 2)] + fill
            nchunk = 8
            cw = S // nchunk
            for n in range(nchunk):
                qt_all[h, :, n * cw:(n + 1) * cw] = _pk(
                    _dot(_ld(wqt[h % 2]), _ld(xbt[:, n * cw:(n + 1) * cw])) * scale)
                for f in fill[len(fill) * n // (nchunk - 1):len(fill) * (n + 1) // (nchunk - 1)]:
                    f()

        def qproj1(h, carry):
            @pl.when(h + 2 < NP)
            def _():
                for cp in q_copies(h + 2):
                    cp.start()

            for cp in a_copies(h):
                cp.start()
            q_head(h, [])
            return carry

        def qproj2(j, carry):
            for cp in rest_copies(j):
                cp.start()

            @pl.when(j == NL // 2)
            def _():
                for cp in kv_copies(0):
                    cp.start()

            for cp in a_copies(j):
                cp.wait()

            def side_by_side(dst, ja, lw, rw0, rw1, mul):
                zero = jnp.zeros((PAD, Dh), BF16)
                ev = _dot_nt(_unpack(lw, 16), jnp.concatenate([rw0, zero], axis=0)) * mul
                od = _dot_nt(_unpack(lw, 0), jnp.concatenate([zero, rw1], axis=0)) * mul
                dst[ja, :, 0:LO] = _pk(ev[:, :LO])
                dst[ja, :, LO:LO + 128] = _pk(ev[:, LO:] + od[:, :128])
                dst[ja, :, LO + 128:] = _pk(od[:, 128:])

            def a_vo(ja):
                side_by_side(wvo, ja, rv[ja], _ld(wot[2 * ja]), _ld(wot[2 * ja + 1]), 1.0)

            def a_kq(ja):
                side_by_side(wkq, ja, rk[ja], _unpack(rq[ja], 16), _unpack(rq[ja], 0), scale)

            def tr():
                n = S // NP
                r0 = _mo(j * n, n)
                xa[pl.ds(_mo(j * (n // 2), n // 2), n // 2), :] = _pk(xat[:, pl.ds(r0, n)].T)

            q_head(j + NL, [tr, functools.partial(a_kq, j), functools.partial(a_vo, j)])
            return carry

        with jax.named_scope('s_qproj'):
            lax.fori_loop(0, NL, qproj1, 0)
            cp_xa.wait()
            lax.fori_loop(0, NL, qproj2, 0)

        with jax.named_scope('s_wait2'):
            for j in range(NL):
                for cp in rest_copies(j):
                    cp.wait()
            for cp in kv_copies(0) + [cp_m]:
                cp.wait()

        KH = KVC // 2
        DH2 = Dc // 2

        def csum(t, carry):
            n, r = t // (KH // 128), t % (KH // 128)
            top = pl.ds(_mo(n * (KVC // 2) + r * 64, 64), 64)
            bot = pl.ds(_mo(n * (KVC // 2) + KH // 2 + r * 64, 64), 64)
            a11, a12 = _ld(c[top, 0:DH2]).astype(F32), _ld(c[top, DH2:]).astype(F32)
            a21, a22 = _ld(c[bot, 0:DH2]).astype(F32), _ld(c[bot, DH2:]).astype(F32)
            dst = pl.ds(_mo(t * 64, 64), 64)
            for i, x in enumerate((a11 + a22, a21 + a22, a11 + a12, a21 - a11, a12 - a22)):
                cs[i, dst, :] = _pk(x)
            return carry

        lax.fori_loop(0, S // 256, csum, 0)

        RH = seg_per_head * seg

        def early_out(h):
            r0 = h * RH if isinstance(h, int) else _mo(h * RH, RH)
            return pltpu.make_async_copy(outv.at[pl.ds(r0, RH), pl.ds(0, LO)],
                                         out_hbm.at[pl.ds(r0, RH), pl.ds(0, LO)], sems.at[11 + h // 8, h % 8])

        memf[...] = mem0[...].astype(F32)
        krow = lax.broadcasted_iota(jnp.int32, (BQ, BQ), 0)
        qcol = lax.broadcasted_iota(jnp.int32, (BQ, BQ), 1)
        cmask = krow <= qcol
        GH = 128 // L
        arow = lax.broadcasted_iota(jnp.int32, (L, 128), 0)
        alane = lax.broadcasted_iota(jnp.int32, (L, 128), 1)
        aseg = sum((alane >= L * i).astype(jnp.int32) for i in range(1, GH + 1))
        acol = alane - L * aseg
        amask = (arow < M) | (arow >= acol)
        NPAIR = H // 2
        groups = [list(range(g, min(g + GH, NPAIR))) for g in range(0, NPAIR, GH)]
        UW = 2 * Dm

        def a_ops(s, st, prev):
            r0 = _mo(s * seg, seg)
            v_ = {}

            def f_k(j):
                if j == 0:
                    xs = _ld(xa[pl.ds(_mo(s * (seg // 2), seg // 2), seg // 2), :]).astype(F32)
                    v_["h"] = jnp.concatenate([st["mem"], xs], axis=0)
                    v_["hodd"] = jnp.concatenate([jnp.zeros((L, PAD), F32), v_["h"]], axis=1)
                v_["k", j] = _dot(v_["h"], _ld(wkq[j]))

            def f_u(j):
                v_["u", j] = _dot(v_["h"], _ld(wvo[j]))

            def rows_at(parts):
                used = sum(p.shape[0] for p in parts)
                pad = [jnp.zeros((128 - used, parts[0].shape[1]), F32)]
                return jnp.concatenate(parts + pad, axis=0).astype(BF16)

            def f_s(g, par):
                if par == 0:
                    sc = _dot_nt(v_["h"], rows_at([v_["k", j][:, :Dm] for j in groups[g]]))
                else:
                    ks = [jnp.concatenate([jnp.where(alane < PAD, 0.0, v_["k", j][:, LO:LO + 128]),
                                           v_["k", j][:, LO + 128:]], axis=1) for j in groups[g]]
                    sc = _dot_nt(v_["hodd"], rows_at(ks))
                n = len(groups[g])
                sc = jnp.where(amask & (aseg < n), sc, NEG)
                m = None
                for i in range(n):
                    mi = jnp.max(jnp.where(aseg == i, sc, -jnp.inf), axis=-1, keepdims=True)
                    m = mi if m is None else jnp.where(aseg == i, mi, m)
                p = jnp.where(aseg < n, jnp.exp2(sc - m), 0.0)
                l = None
                for i in range(n):
                    li = jnp.sum(jnp.where(aseg == i, p, 0.0), axis=-1, keepdims=True)
                    l = li if l is None else jnp.where(aseg == i, li, l)
                v_["p", g, par] = p / l

            def f_o(g, par):
                c0 = par * LO
                d = _dot(v_.pop(("p", g, par)), rows_at([v_["u", j][:, c0:c0 + Dm + PAD] for j in groups[g]]))
                v_["acc", par] = d if g == 0 else v_["acc", par] + d
                if g == len(groups) - 1 and par == 1:
                    o = v_["acc", 0][:, :Dm] + v_["acc", 1][:, PAD:]
                    outv[pl.ds(r0, seg), 0:Dm] = o[M:, :].astype(BF16)
                    st["mem"] = o[:M, :]

            P = functools.partial
            kk = [_Op("k%d" % j, 280, [(prev, LAT_M)] if (j == 0 and prev) else [], P(f_k, j)) for j in range(NPAIR)]
            uu = [_Op("u%d" % j, 280, [], P(f_u, j)) for j in range(NPAIR)]
            q = []
            pend = []
            for g, prs in enumerate(groups):
                for j in prs:
                    q.append(kk[j])
                    q += pend
                    pend = []
                q.append(uu[prs[0]])
                ss = [_Op("s", 40, [(kk[prs[-1]], LAT_S)], P(f_s, g, par)) for par in range(2)]
                q += ss
                q += [uu[j] for j in prs[1:]]
                pend = [_Op("o", 40, [(ss[par], LAT_O), (uu[prs[-1]], LAT_R)], P(f_o, g, par)) for par in range(2)]
            return q + pend

        def b_ops(h):
            v_ = {}
            KT = KC // BQ

            def chunks(i):
                return [(t0, min(t0 + KT, i + 1)) for t0 in range(0, i + 1, KT)]

            def f_qk(i, t0, t1):
                qt = _ld(qt_all[h, :, BQ * i:BQ * (i + 1)])
                k0, k1 = BQ * t0, BQ * t1
                km = (k0 + k1) // 2
                sc = jnp.concatenate([_dot(_ld(kh[k0 // 2:km // 2, :]), qt), _dot(_ld(kh[km // 2:k1 // 2, :]), qt)], axis=0)
                if t1 == i + 1:
                    sd = jnp.where(cmask, sc[k1 - k0 - BQ:, :], NEG)
                    sc = jnp.concatenate([sc[:k1 - k0 - BQ, :], sd], axis=0) if t1 - t0 > 1 else sd
                v_["s", i, t0] = sc
                m = jnp.max(sc.reshape((k1 - k0) // RM, RM, BQ), axis=0)
                v_["m", i] = m if t0 == 0 else jnp.maximum(v_["m", i], m)
                if t1 == i + 1:
                    v_["m", i] = jnp.max(v_["m", i], axis=0, keepdims=True)

            def f_e(i, t0, t1, e0, e1):
                p = jnp.exp2(v_["s", i, t0][e0:e1, :] - v_["m", i])
                l = jnp.sum(p.reshape((e1 - e0) // RS, RS, BQ), axis=0)
                v_["l", i] = l if (t0 == 0 and e0 == 0) else v_["l", i] + l
                v_.setdefault(("p", i, t0), []).append(p.astype(BF16))

            def f_pv(i, t0, t1):
                p = jnp.concatenate(v_.pop(("p", i, t0)), axis=0)
                ns = {0: 1, 1: 4, 2: 2, 3: 4}[(t1 - t0) % 4]
                rr = Dh // ns
                d = jnp.concatenate([_dot(_ld(vth[r * rr // 2:(r + 1) * rr // 2, BQ * t0:BQ * t1]), p) for r in range(ns)], axis=0)
                v_["c", i] = d if t0 == 0 else v_["c", i] + d
                if t1 == i + 1:
                    r = 1.0 / jnp.sum(v_.pop(("l", i)), axis=0, keepdims=True)
                    v_["c", i] = (v_["c", i] * r).astype(BF16)

            def f_op(i):
                ct = v_.pop(("c", i))
                hm = Dm // 2
                for r in range(2):
                    acct[PAD + r * hm:PAD + (r + 1) * hm, BQ * i:BQ * (i + 1)] += _dot(
                        _ld(bwot[h, r * hm // 2:(r + 1) * hm // 2, :]), ct)

            P = functools.partial
            qk = [[_Op("QK%d" % i, 64 * (t1 - t0), [], P(f_qk, i, t0, t1)) for t0, t1 in chunks(i)]
                  for i in range(nqb)]
            epv = []
            for i in range(nqb):
                es = [[_Op("E", 0, [(qk[i][-1], LAT_BP)], P(f_e, i, t0, t1, e0, min(e0 + EC, BQ * (t1 - t0))))
                       for e0 in range(0, BQ * (t1 - t0), EC)] for t0, t1 in chunks(i)]
                pv = [_Op("PV%d" % i, 64 * (t1 - t0), [(es[n][-1], LAT_BE)], P(f_pv, i, t0, t1))
                      for n, (t0, t1) in enumerate(chunks(i))]
                l = list(es[0])
                for n in range(len(pv)):
                    if n + 1 < len(pv):
                        l += es[n + 1]
                    l.append(pv[n])
                epv.append(l)
            op = [_Op("OP%d" % i, 224, [(epv[i][-1], LAT_BO)], P(f_op, i)) for i in range(nqb)]
            q = []
            order = ORDER(nqb)
            for t in range(nqb + 2):
                l1 = qk[order[t]] if t < nqb else []
                l2 = epv[order[t - 1]] if 0 <= t - 1 < nqb else []
                keyed = [((n + 0.25) / len(l1), 0, o) for n, o in enumerate(l1)]
                keyed += [((n + 0.75) / len(l2), 1, o) for n, o in enumerate(l2)]
                q += [o for _, _, o in sorted(keyed, key=lambda z: z[:2])]
                if 0 <= t - 2 < nqb:
                    q.append(op[order[t - 2]])
            return q

        def head(h, carry):
            if DO_B:
                shift = (16 * (1 - h % 2)).astype(U32)
                with jax.named_scope('s_kv'):
                    def kvb(n, carry):
                        def wcombos(w11, w12, w21, w22):
                            f = lambda x: x.astype(BF16)
                            return [f(w11 + w22), f(w11), f(w12 - w22), f(w21 - w11), f(w22), f(w11 + w12),
                                    f(w21 + w22)]

                        def lhs(p, r, m):
                            if p == 2:
                                return _ld(c[pl.ds(_mo(n * (KVC // 2) + r // 2, 8), m // 2), 0:DH2])
                            if p == 3:
                                return _ld(c[pl.ds(_mo(n * (KVC // 2) + (KH + r) // 2, 8), m // 2), DH2:])
                            return _ld(cs[(0, 1, None, None, 2, 3, 4)[p],
                                          pl.ds(_mo(n * (KH // 2) + r // 2, 8), m // 2), :])

                        def outs(m):
                            return (m[0] + m[3] - m[4] + m[6], m[2] + m[4], m[1] + m[3], m[0] - m[1] + m[2] + m[5])

                        wk = _unpack_f32(ruk[h // 2], shift)
                        wc = wcombos(wk[:DH2, :128], wk[:DH2, 128:], wk[DH2:, :128], wk[DH2:, 128:])
                        for r in range(0, KH, KM):
                            c11, c12, c21, c22 = outs([_dot(lhs(p, r, KM), wc[p]) for p in range(7)])
                            top = pl.ds(_mo(n * (KVC // 2) + r // 2, 8), KM // 2)
                            bot = pl.ds(_mo(n * (KVC // 2) + (KH + r) // 2, 8), KM // 2)
                            kh[top, 0:128] = _pk(c11)
                            kh[top, 128:] = _pk(c12)
                            kh[bot, 0:128] = _pk(c21)
                            kh[bot, 128:] = _pk(c22)
                        wv = _unpack_f32(ruv[h // 2].T, shift)
                        wc = wcombos(wv[:128, :DH2], wv[128:, :DH2], wv[:128, DH2:], wv[128:, DH2:])
                        for r in range(0, KH, 128):
                            c11, c12, c21, c22 = outs([_dot_nt(wc[p], lhs(p, r, 128)) for p in range(7)])
                            top = pl.ds(_mo(n * KVC + r, 128), 128)
                            bot = pl.ds(_mo(n * KVC + KH + r, 128), 128)
                            vth[0:64, top] = _pk(c11)
                            vth[64:, top] = _pk(c12)
                            vth[0:64, bot] = _pk(c21)
                            vth[64:, bot] = _pk(c22)
                        return carry
                    if KVLOOP:
                        lax.fori_loop(0, S // KVC, kvb, 0)
                    else:
                        for n in range(S // KVC):
                            kvb(n, 0)

            @pl.when((h % 2 == 0) & (h < H - 2))
            def _():
                for cp in kv_copies(h // 2 + 1):
                    cp.start()

            @pl.when((h % 2 == 1) & (h < H - 1))
            def _():
                for cp in kv_copies(h // 2 + 1):
                    cp.wait()

            @pl.when(h > 0)
            def _():
                early_out(h - 1).start()

            st = {"mem": memf[...]}
            qa = []
            if DO_A:
                for t in range(seg_per_head):
                    qa += a_ops(h * seg_per_head + t, st, qa[-1] if qa else None)
            qb = b_ops(h) if DO_B else []
            with jax.named_scope('s_att'):
                for o in _merge(qa, qb):
                    o.fn()
            memf[...] = st["mem"]
            return carry

        with jax.named_scope('s_heads'):
            lax.fori_loop(0, H, head, 0)

        def out_copy(r):
            r0 = _mo(r * OB, OB)
            return pltpu.make_async_copy(outv.at[pl.ds(r0, OB), pl.ds(LO, 2 * Dm - LO)],
                                         out_hbm.at[pl.ds(r0, OB), pl.ds(LO, 2 * Dm - LO)], sems.at[7, r])

        def epi(r, carry):
            lane = lax.broadcasted_iota(jnp.int32, (OB, 128), 1)
            rows = pl.ds(_mo(r * OB, OB), OB)
            bt = acct[:, rows].T.astype(BF16)
            outv[rows, LO:LO + 128] = jnp.where(lane < 128 - PAD, outv[rows, LO:LO + 128], bt[:, 0:128])
            outv[rows, LO + 128:] = bt[:, 128:]
            out_copy(r).start()
            return carry

        with jax.named_scope('s_epi'):
            early_out(H - 1).start()
            lax.fori_loop(0, S // OB, epi, 0)
            for hh in range(H):
                early_out(hh).wait()
            for r in range(S // OB):
                out_copy(r).wait()

    return kernel


@functools.partial(jax.jit, static_argnames=("A_seg_len",))
def pallas_concat_heads__memory_aug_recurrent_mem_tr__compressed_kv_cla__prompt_kernel(A_x, A_mem0, A_Wq, A_Wk, A_Wv, A_Wo, A_seg_len, B_x, B_c_kv, B_w_q, B_w_uk, B_w_uv, B_w_o):
    _, S, Dm = A_x.shape
    M = A_mem0.shape[1]
    H, Dh = A_Wq.shape[1], A_Wq.shape[2]
    Dc = B_c_kv.shape[2]
    seg = int(A_seg_len)
    kern = _make_kernel(S, Dm, H, Dh, M, seg, Dc)
    any_spec = pl.BlockSpec(memory_space=pl.ANY)
    scratch = [
        pltpu.VMEM((Dm, S), BF16),
        pltpu.VMEM((S // 2, Dm), U32),
        pltpu.VMEM((M, Dm), BF16),
        pltpu.VMEM((H // 2, Dm, Dh), U32),
        pltpu.VMEM((H // 2, Dm, Dh), U32),
        pltpu.VMEM((H // 2, Dm, Dh), U32),
        pltpu.VMEM((H // 2, Dm // 2, 2 * Dm), U32),
        pltpu.VMEM((H // 2, Dm // 2, 2 * Dm), U32),
        pltpu.VMEM((H, Dm // 2, Dh), U32),
        pltpu.VMEM((Dm // 2, S), U32),
        pltpu.VMEM((S // 2, Dc), U32),
        pltpu.VMEM((H // 2, Dm, Dh), U32),
        pltpu.VMEM((H // 2, Dc, Dh), U32),
        pltpu.VMEM((H // 2, Dc, Dh), U32),
        pltpu.VMEM((H, Dm // 2, Dh), U32),
        pltpu.VMEM((H, Dh // 2, S), U32),
        pltpu.VMEM((5, S // 4, Dc // 2), U32),
        pltpu.VMEM((2, Dh // 2, Dm), U32),
        pltpu.VMEM((M, Dm), F32),
        pltpu.VMEM((S // 2, Dh), U32),
        pltpu.VMEM((Dh // 2, S), U32),
        pltpu.VMEM((Dm + (-Dm) % 128, S), F32),
        pltpu.VMEM((S, 2 * Dm), BF16),
        pltpu.SemaphoreType.DMA((13, 8)),
    ]
    out = pl.pallas_call(
        kern,
        out_shape=jax.ShapeDtypeStruct((S, 2 * Dm), BF16),
        in_specs=[any_spec] * 12,
        out_specs=any_spec,
        scratch_shapes=scratch,
        compiler_params=pltpu.CompilerParams(vmem_limit_bytes=120 * 1024 * 1024),
    )(A_x[0].T, A_mem0.reshape(M, Dm), A_Wq, A_Wk, A_Wv, jnp.swapaxes(A_Wo, 1, 2),
      B_x[0].T, B_c_kv.reshape(S, Dc), B_w_q, B_w_uk, B_w_uv, jnp.swapaxes(B_w_o, 1, 2))
    return out.reshape(1, S, 2 * Dm)
```

```python
import functools
import jax
import jax.numpy as jnp
import numpy as np
from jax import lax
from jax.experimental import pallas as pl
from jax.experimental.pallas import tpu as pltpu

F32 = jnp.float32
BF16 = jnp.bfloat16
U32 = jnp.uint32

LOG2E = 1.4426950408889634
NEG = -1000000000.0 * LOG2E

KC = 256
EC = 128
RM = 32
RS = 32
KVC = 1024
KM = 128
OB = 256

BIAS = 0.005
OPD = 6
LAT_S = 250
LAT_O = 350
LAT_R = 200
LAT_M = 350
LAT_BP = 200
LAT_BE = 150
LAT_BO = 250


def _dot(a, b):
    return lax.dot_general(a, b, (((1,), (0,)), ((), ())), preferred_element_type=F32)


def _dot_nt(a, b):
    return lax.dot_general(a, b, (((1,), (1,)), ((), ())), preferred_element_type=F32)


def _unpack(u, shift):
    w = (u << shift) & jnp.uint32(0xFFFF0000)
    return pltpu.bitcast(w, F32).astype(BF16)


def _unpack_f32(u, shift):
    return pltpu.bitcast((u << shift) & jnp.uint32(0xFFFF0000), F32)


def _mo(i, n):
    return i if isinstance(i, int) else pl.multiple_of(i, n)


def _ld(words):
    return pltpu.bitcast(words, BF16)


def _pk(x):
    return pltpu.bitcast(x.astype(BF16), U32)


class _Op:
    def __init__(self, name, cost, deps, fn):
        self.name, self.cost, self.deps, self.fn = name, cost, deps, fn
        self.end = None


def _merge(qa, qb):
    ta = sum(o.cost for o in qa) or 1
    tb = sum(o.cost for o in qb) or 1
    ia = ib = 0
    da = db = 0
    t = 0
    order = []

    def ready(o):
        return max([0] + [d.end + lat for d, lat in o.deps])

    while ia < len(qa) or ib < len(qb):
        cand = []
        if ia < len(qa):
            cand.append((max(ready(qa[ia]), t), da / ta, 0))
        if ib < len(qb):
            cand.append((max(ready(qb[ib]), t), db / tb + BIAS, 1))
        st, _, w = min(cand)
        o = qa[ia] if w == 0 else qb[ib]
        t = st + o.cost
        o.end = t
        order.append(o)
        if w == 0:
            ia += 1
            da += o.cost
        else:
            ib += 1
            db += o.cost
    return order


def _make_kernel(S, Dm, H, Dh, M, seg, Dc):
    n_seg = S // seg
    seg_per_head = n_seg // H
    L = M + seg
    BQ = 128
    nqb = S // BQ
    scale = Dh ** (-0.5) * LOG2E
    PAD = (-Dm) % 128
    LO = Dm + PAD - 128

    def kernel(xat_hbm, mem0_hbm, wq_hbm, wk_hbm, wv_hbm, wot_hbm,
               xbt_hbm, c_hbm, bwq_hbm, wuk_hbm, wuv_hbm, bwot_hbm,
               out_hbm,
               xat, xa, mem0, rq, rk, rv, wkq, wvo, wot,
               xbt, c, rbq, ruk, ruv, bwot,
               qt_all, cs, wqt, memf, kh, vth, acct, outv, sems):

        NP = H // 2

        def pcopy(src, dst, j, s0):
            return pltpu.make_async_copy(src.bitcast(U32).at[:, j, :], dst.at[j], sems.at[s0, j])

        def q_copies(j):
            return [pcopy(bwq_hbm, rbq, j, 0)]

        def a_copies(j):
            return [pcopy(wq_hbm, rq, j, 1), pcopy(wk_hbm, rk, j, 2), pcopy(wv_hbm, rv, j, 3),
                    pltpu.make_async_copy(wot_hbm.bitcast(U32).at[pl.ds(2 * j, 2)], wot.at[pl.ds(2 * j, 2)],
                                          sems.at[9, j])]

        def kv_copies(j):
            return [pcopy(wuk_hbm, ruk, j, 4), pcopy(wuv_hbm, ruv, j, 5)]

        cp_x = pltpu.make_async_copy(xbt_hbm.bitcast(U32), xbt, sems.at[6, 0])
        cp_xa = pltpu.make_async_copy(xat_hbm, xat, sems.at[6, 1])
        cp_m = pltpu.make_async_copy(mem0_hbm, mem0, sems.at[6, 3])
        NL = H // 2
        HL = H // NL

        def c_copies(t):
            n, r = t // (KVC // 256), t % (KVC // 256)
            cps = []
            for half in range(2):
                rows = pl.ds(_mo(n * (KVC // 2) + half * (KVC // 4) + r * 64, 64), 64)
                cps.append(pltpu.make_async_copy(c_hbm.bitcast(U32).at[rows], c.at[rows], sems.at[8 + 5 * half, t]))
            return cps

        def rest_copies(j):
            return [pltpu.make_async_copy(bwot_hbm.bitcast(U32).at[pl.ds(HL * j, HL)], bwot.at[pl.ds(HL * j, HL)],
                                          sems.at[10, j])]

        for cp in q_copies(0) + [cp_x] + q_copies(1):
            cp.start()

        def zero(r, carry):
            acct[:, pl.ds(_mo(r * 128, 128), 128)] = jnp.zeros((acct.shape[0], 128), F32)
            return carry

        lax.fori_loop(0, S // 128, zero, 0)

        def q_weights(h, slot):
            wqt[slot] = _pk(_unpack(rbq[h // 2].T, (16 * (1 - h % 2)).astype(U32)))

        for cp in q_copies(0):
            cp.wait()
        q_weights(jnp.int32(0), 0)
        cp_x.wait()
        cp_xa.start()
        cp_m.start()

        def q_head(h, fill):
            @pl.when((h % 2 == 1) & (h + 1 < H))
            def _():
                for cp in q_copies((h + 1) // 2):
                    cp.wait()

            fill = [functools.partial(q_weights, jnp.minimum(h + 1, H - 1), (h + 1) % 2)] + fill
            nchunk = 8
            cw = S // nchunk
            for n in range(nchunk):
                qt_all[h, :, n * cw:(n + 1) * cw] = _pk(
                    _dot(_ld(wqt[h % 2]), _ld(xbt[:, n * cw:(n + 1) * cw])) * scale)
                for f in fill[len(fill) * n // (nchunk - 1):len(fill) * (n + 1) // (nchunk - 1)]:
                    f()

        KH = KVC // 2
        DH2 = Dc // 2

        def csum(t):
            n, r = t // (KH // 128), t % (KH // 128)
            top = pl.ds(_mo(n * (KVC // 2) + r * 64, 64), 64)
            bot = pl.ds(_mo(n * (KVC // 2) + KH // 2 + r * 64, 64), 64)
            dst = pl.ds(_mo(t * 64, 64), 64)
            blocks = (c[top, 0:DH2], c[top, DH2:], c[bot, 0:DH2], c[bot, DH2:])
            sums = []
            for par in range(2):
                a11, a12, a21, a22 = (_unpack_f32(x, 16 * (1 - par)) for x in blocks)
                sums.append((a11 + a22, a21 + a22, a11 + a12, a21 - a11, a12 - a22))
            for i, (lo, hi) in enumerate(zip(*sums)):
                cs[i, dst, :] = pltpu.bitcast(pltpu.pack_elementwise([lo, hi], packed_dtype=BF16), U32)

        def qproj1(h, carry):
            @pl.when(h + 2 < NP)
            def _():
                for cp in q_copies(h + 2):
                    cp.start()

            @pl.when(h + 2 == NP)
            def _():
                for cp in c_copies(0):
                    cp.start()

            for cp in a_copies(h):
                cp.start()
            q_head(h, [])
            return carry

        def qproj2(j, carry):
            for cp in rest_copies(j):
                cp.start()

            @pl.when(j + 1 < NL)
            def _():
                for cp in c_copies(j + 1):
                    cp.start()

            @pl.when(j == NL // 2)
            def _():
                for cp in kv_copies(0):
                    cp.start()

            for cp in a_copies(j) + c_copies(j):
                cp.wait()

            def side_by_side(dst, ja, lw, rw0, rw1, mul):
                zero = jnp.zeros((PAD, Dh), BF16)
                ev = _dot_nt(_unpack(lw, 16), jnp.concatenate([rw0, zero], axis=0)) * mul
                od = _dot_nt(_unpack(lw, 0), jnp.concatenate([zero, rw1], axis=0)) * mul
                dst[ja, :, 0:LO] = _pk(ev[:, :LO])
                dst[ja, :, LO:LO + 128] = _pk(ev[:, LO:] + od[:, :128])
                dst[ja, :, LO + 128:] = _pk(od[:, 128:])

            def a_vo(ja):
                side_by_side(wvo, ja, rv[ja], _ld(wot[2 * ja]), _ld(wot[2 * ja + 1]), 1.0)

            def a_kq(ja):
                side_by_side(wkq, ja, rk[ja], _unpack(rq[ja], 16), _unpack(rq[ja], 0), scale)

            def tr():
                n = S // NP
                r0 = _mo(j * n, n)
                xa[pl.ds(_mo(j * (n // 2), n // 2), n // 2), :] = _pk(xat[:, pl.ds(r0, n)].T)

            q_head(j + NL, [tr] + [functools.partial(f, j) for f in (csum, a_kq, a_vo)])
            return carry

        lax.fori_loop(0, NL, qproj1, 0)
        cp_xa.wait()
        lax.fori_loop(0, NL, qproj2, 0)

        for j in range(NL):
            for cp in rest_copies(j):
                cp.wait()
        for cp in kv_copies(0) + [cp_m]:
            cp.wait()

        RH = seg_per_head * seg

        def early_out(h):
            r0 = h * RH if isinstance(h, int) else _mo(h * RH, RH)
            return pltpu.make_async_copy(outv.at[pl.ds(r0, RH), pl.ds(0, LO)],
                                         out_hbm.at[pl.ds(r0, RH), pl.ds(0, LO)], sems.at[11 + h // 8, h % 8])

        memf[...] = mem0[...].astype(F32)
        krow = lax.broadcasted_iota(jnp.int32, (BQ, BQ), 0)
        qcol = lax.broadcasted_iota(jnp.int32, (BQ, BQ), 1)
        cmask = krow <= qcol
        GH = 128 // L
        arow = lax.broadcasted_iota(jnp.int32, (L, 128), 0)
        alane = lax.broadcasted_iota(jnp.int32, (L, 128), 1)
        aseg = sum((alane >= L * i).astype(jnp.int32) for i in range(1, GH + 1))
        acol = alane - L * aseg
        amask = (arow < M) | (arow >= acol)
        NPAIR = H // 2
        groups = [list(range(g, min(g + GH, NPAIR))) for g in range(0, NPAIR, GH)]

        def a_ops(s, st, prev):
            r0 = _mo(s * seg, seg)
            v_ = {}

            def f_k(j):
                if j == 0:
                    xs = _ld(xa[pl.ds(_mo(s * (seg // 2), seg // 2), seg // 2), :]).astype(F32)
                    v_["h"] = jnp.concatenate([st["mem"], xs], axis=0)
                    v_["hodd"] = jnp.concatenate([jnp.zeros((L, PAD), F32), v_["h"]], axis=1)
                v_["k", j] = _dot(v_["h"], _ld(wkq[j]))

            def f_u(j):
                v_["u", j] = _dot(v_["h"], _ld(wvo[j]))

            def rows_at(parts):
                used = sum(p.shape[0] for p in parts)
                pad = [jnp.zeros((128 - used, parts[0].shape[1]), F32)]
                return jnp.concatenate(parts + pad, axis=0).astype(BF16)

            def f_s(g, par):
                if par == 0:
                    sc = _dot_nt(v_["h"], rows_at([v_["k", j][:, :Dm] for j in groups[g]]))
                else:
                    ks = [jnp.concatenate([jnp.where(alane < PAD, 0.0, v_["k", j][:, LO:LO + 128]),
                                           v_["k", j][:, LO + 128:]], axis=1) for j in groups[g]]
                    sc = _dot_nt(v_["hodd"], rows_at(ks))
                n = len(groups[g])
                sc = jnp.where(amask & (aseg < n), sc, NEG)
                m = None
                for i in range(n):
                    mi = jnp.max(jnp.where(aseg == i, sc, -jnp.inf), axis=-1, keepdims=True)
                    m = mi if m is None else jnp.where(aseg == i, mi, m)
                p = jnp.where(aseg < n, jnp.exp2(sc - m), 0.0)
                l = None
                for i in range(n):
                    li = jnp.sum(jnp.where(aseg == i, p, 0.0), axis=-1, keepdims=True)
                    l = li if l is None else jnp.where(aseg == i, li, l)
                v_["p", g, par] = p / l

            def f_o(g, par):
                c0 = par * LO
                d = _dot(v_.pop(("p", g, par)), rows_at([v_["u", j][:, c0:c0 + Dm + PAD] for j in groups[g]]))
                v_["acc", par] = d if g == 0 else v_["acc", par] + d
                if g == len(groups) - 1 and par == 1:
                    o = v_["acc", 0][:, :Dm] + v_["acc", 1][:, PAD:]
                    outv[pl.ds(r0, seg), 0:Dm] = o[M:, :].astype(BF16)
                    st["mem"] = o[:M, :]

            P = functools.partial
            kk = [_Op("k%d" % j, 280, [(prev, LAT_M)] if (j == 0 and prev) else [], P(f_k, j)) for j in range(NPAIR)]
            uu = [_Op("u%d" % j, 280, [], P(f_u, j)) for j in range(NPAIR)]
            q = []
            pend = []
            for g, prs in enumerate(groups):
                for j in prs:
                    q.append(kk[j])
                    q += pend
                    pend = []
                q.append(uu[prs[0]])
                ss = [_Op("s", 40, [(kk[prs[-1]], LAT_S)], P(f_s, g, par)) for par in range(2)]
                q += ss
                q += [uu[j] for j in prs[1:]]
                pend = [_Op("o", 40, [(ss[par], LAT_O), (uu[prs[-1]], LAT_R)], P(f_o, g, par)) for par in range(2)]
            return q + pend

        def b_ops(h):
            v_ = {}
            KT = KC // BQ

            def chunks(i):
                return [(t0, min(t0 + KT, i + 1)) for t0 in range(0, i + 1, KT)]

            def f_qk(i, t0, t1):
                qt = _ld(qt_all[h, :, BQ * i:BQ * (i + 1)])
                k0, k1 = BQ * t0, BQ * t1
                km = (k0 + k1) // 2
                sc = jnp.concatenate([_dot(_ld(kh[k0 // 2:km // 2, :]), qt), _dot(_ld(kh[km // 2:k1 // 2, :]), qt)], axis=0)
                if t1 == i + 1:
                    sd = jnp.where(cmask, sc[k1 - k0 - BQ:, :], NEG)
                    sc = jnp.concatenate([sc[:k1 - k0 - BQ, :], sd], axis=0) if t1 - t0 > 1 else sd
                v_["s", i, t0] = sc
                m = jnp.max(sc.reshape((k1 - k0) // RM, RM, BQ), axis=0)
                v_["m", i] = m if t0 == 0 else jnp.maximum(v_["m", i], m)
                if t1 == i + 1:
                    v_["m", i] = jnp.max(v_["m", i], axis=0, keepdims=True)

            def f_e(i, t0, t1, e0, e1):
                p = jnp.exp2(v_["s", i, t0][e0:e1, :] - v_["m", i])
                l = jnp.sum(p.reshape((e1 - e0) // RS, RS, BQ), axis=0)
                v_["l", i] = l if (t0 == 0 and e0 == 0) else v_["l", i] + l
                v_.setdefault(("p", i, t0), []).append(p.astype(BF16))

            def f_pv(i, t0, t1):
                p = jnp.concatenate(v_.pop(("p", i, t0)), axis=0)
                ns = {0: 1, 1: 4, 2: 2, 3: 4}[(t1 - t0) % 4]
                rr = Dh // ns
                d = jnp.concatenate([_dot(_ld(vth[r * rr // 2:(r + 1) * rr // 2, BQ * t0:BQ * t1]), p) for r in range(ns)], axis=0)
                v_["c", i] = d if t0 == 0 else v_["c", i] + d
                if t1 == i + 1:
                    r = 1.0 / jnp.sum(v_.pop(("l", i)), axis=0, keepdims=True)
                    v_["c", i] = v_["c", i] * r

            hm = Dm // 2

            def f_wo():
                w = _ld(bwot[h]).astype(F32)
                w11, w12, w21, w22 = w[:hm, :128], w[:hm, 128:], w[hm:, :128], w[hm:, 128:]
                v_["wo"] = [x.astype(BF16)
                            for x in (w11 + w22, w21 + w22, w11, w22, w11 + w12, w21 - w11, w12 - w22)]

            def f_op(i):
                c0, c1 = v_.pop(("c", i)), v_.pop(("c", i + 1))
                cc = wcombos(c0[:128], c1[:128], c0[128:], c1[128:])
                o11, o12, o21, o22 = outs([_dot(v_["wo"][p], cc[p]) for p in range(7)])
                acct[PAD:PAD + hm, BQ * i:BQ * (i + 1)] += o11
                acct[PAD:PAD + hm, BQ * (i + 1):BQ * (i + 2)] += o12
                acct[PAD + hm:, BQ * i:BQ * (i + 1)] += o21
                acct[PAD + hm:, BQ * (i + 1):BQ * (i + 2)] += o22

            shift = (16 * (1 - h % 2)).astype(U32)

            def wcombos(w11, w12, w21, w22):
                return [x.astype(BF16) for x in (w11 + w22, w11, w12 - w22, w21 - w11, w22, w11 + w12, w21 + w22)]

            def lhs(p, n, r):
                if p == 2:
                    return _ld(c[(n * KVC + r) // 2:(n * KVC + r + KM) // 2, 0:DH2])
                if p == 3:
                    return _ld(c[(n * KVC + KH + r) // 2:(n * KVC + KH + r + KM) // 2, DH2:])
                return _ld(cs[(0, 1, None, None, 2, 3, 4)[p], (n * KH + r) // 2:(n * KH + r + KM) // 2, :])

            def outs(m):
                return (m[0] + m[3] - m[4] + m[6], m[2] + m[4], m[1] + m[3], m[0] - m[1] + m[2] + m[5])

            def f_kp(n, r):
                if "wk" not in v_:
                    w = _unpack_f32(ruk[h // 2], shift)
                    v_["wk"] = wcombos(w[:DH2, :128], w[:DH2, 128:], w[DH2:, :128], w[DH2:, 128:])
                c11, c12, c21, c22 = outs([_dot(lhs(p, n, r), v_["wk"][p]) for p in range(7)])
                top = slice((n * KVC + r) // 2, (n * KVC + r + KM) // 2)
                bot = slice((n * KVC + KH + r) // 2, (n * KVC + KH + r + KM) // 2)
                kh[top, 0:128] = _pk(c11)
                kh[top, 128:] = _pk(c12)
                kh[bot, 0:128] = _pk(c21)
                kh[bot, 128:] = _pk(c22)

            def f_vp(n, r):
                if "wv" not in v_:
                    w = _unpack_f32(ruv[h // 2].T, shift)
                    v_["wv"] = wcombos(w[:128, :DH2], w[128:, :DH2], w[:128, DH2:], w[128:, DH2:])
                c11, c12, c21, c22 = outs([_dot_nt(v_["wv"][p], lhs(p, n, r)) for p in range(7)])
                top = slice(n * KVC + r, n * KVC + r + KM)
                bot = slice(n * KVC + KH + r, n * KVC + KH + r + KM)
                vth[0:64, top] = _pk(c11)
                vth[64:, top] = _pk(c12)
                vth[0:64, bot] = _pk(c21)
                vth[64:, bot] = _pk(c22)

            P = functools.partial
            nr = [(n, r) for n in range(S // KVC) for r in range(0, KH, KM)]
            kp = [_Op("K", 7 * KM, [], P(f_kp, n, r)) for n, r in nr]
            vp = [_Op("V", 7 * KM, [], P(f_vp, n, r)) for n, r in nr]
            qk = [[_Op("QK%d" % i, 64 * (t1 - t0), [], P(f_qk, i, t0, t1)) for t0, t1 in chunks(i)]
                  for i in range(nqb)]
            epv = []
            for i in range(nqb):
                es = [[_Op("E", 0, [(qk[i][-1], LAT_BP)], P(f_e, i, t0, t1, e0, min(e0 + EC, BQ * (t1 - t0))))
                       for e0 in range(0, BQ * (t1 - t0), EC)] for t0, t1 in chunks(i)]
                pv = [_Op("PV%d" % i, 64 * (t1 - t0), [(es[n][-1], LAT_BE)], P(f_pv, i, t0, t1))
                      for n, (t0, t1) in enumerate(chunks(i))]
                l = list(es[0])
                for n in range(len(pv)):
                    if n + 1 < len(pv):
                        l += es[n + 1]
                    l.append(pv[n])
                epv.append(l)
            op = {i: _Op("OP%d" % i, 392, [(epv[i][-1], LAT_BO), (epv[i + 1][-1], LAT_BO)], P(f_op, i)) for i in range(0, nqb, 2)}
            q = kp[:4] + [_Op('W', 0, [], f_wo)] + kp[4:] + vp[:1]
            order = list(range(nqb - 1, -1, -1))
            for t in range(nqb + OPD):
                l1 = qk[order[t]] if t < nqb else []
                l2 = epv[order[t - 1]] if 0 <= t - 1 < nqb else (vp[1:] if t == 0 else [])
                keyed = [((n + 0.25) / len(l1), 0, o) for n, o in enumerate(l1)]
                keyed += [((n + 0.75) / len(l2), 1, o) for n, o in enumerate(l2)]
                q += [o for _, _, o in sorted(keyed, key=lambda z: z[:2])]
                if 0 <= t - OPD < nqb and (t - OPD) % 2 == 1:
                    q.append(op[order[t - OPD] // 2 * 2])
            return q

        def head(h, carry):
            @pl.when((h % 2 == 0) & (h < H - 2))
            def _():
                for cp in kv_copies(h // 2 + 1):
                    cp.start()

            @pl.when((h % 2 == 1) & (h < H - 1))
            def _():
                for cp in kv_copies(h // 2 + 1):
                    cp.wait()

            @pl.when(h > 0)
            def _():
                early_out(h - 1).start()

            st = {"mem": memf[...]}
            qa = []
            for t in range(seg_per_head):
                qa += a_ops(h * seg_per_head + t, st, qa[-1] if qa else None)
            qb = b_ops(h)
            for o in _merge(qa, qb):
                o.fn()
            memf[...] = st["mem"]
            return carry

        lax.fori_loop(0, H, head, 0)

        def out_copy(r):
            r0 = _mo(r * OB, OB)
            return pltpu.make_async_copy(outv.at[pl.ds(r0, OB), pl.ds(LO, 2 * Dm - LO)],
                                         out_hbm.at[pl.ds(r0, OB), pl.ds(LO, 2 * Dm - LO)], sems.at[7, r])

        def epi(r, carry):
            lane = lax.broadcasted_iota(jnp.int32, (OB, 128), 1)
            rows = pl.ds(_mo(r * OB, OB), OB)
            bt = acct[:, rows].T.astype(BF16)
            outv[rows, LO:LO + 128] = jnp.where(lane < 128 - PAD, outv[rows, LO:LO + 128], bt[:, 0:128])
            outv[rows, LO + 128:] = bt[:, 128:]
            out_copy(r).start()
            return carry

        early_out(H - 1).start()
        lax.fori_loop(0, S // OB, epi, 0)
        for hh in range(H):
            early_out(hh).wait()
        for r in range(S // OB):
            out_copy(r).wait()

    return kernel


@functools.partial(jax.jit, static_argnames=("A_seg_len",))
def pallas_concat_heads__memory_aug_recurrent_mem_tr__compressed_kv_cla__prompt_kernel(A_x, A_mem0, A_Wq, A_Wk, A_Wv, A_Wo, A_seg_len, B_x, B_c_kv, B_w_q, B_w_uk, B_w_uv, B_w_o):
    _, S, Dm = A_x.shape
    M = A_mem0.shape[1]
    H, Dh = A_Wq.shape[1], A_Wq.shape[2]
    Dc = B_c_kv.shape[2]
    seg = int(A_seg_len)
    kern = _make_kernel(S, Dm, H, Dh, M, seg, Dc)
    any_spec = pl.BlockSpec(memory_space=pl.ANY)
    scratch = [
        pltpu.VMEM((Dm, S), BF16),
        pltpu.VMEM((S // 2, Dm), U32),
        pltpu.VMEM((M, Dm), BF16),
        pltpu.VMEM((H // 2, Dm, Dh), U32),
        pltpu.VMEM((H // 2, Dm, Dh), U32),
        pltpu.VMEM((H // 2, Dm, Dh), U32),
        pltpu.VMEM((H // 2, Dm // 2, 2 * Dm), U32),
        pltpu.VMEM((H // 2, Dm // 2, 2 * Dm), U32),
        pltpu.VMEM((H, Dm // 2, Dh), U32),
        pltpu.VMEM((Dm // 2, S), U32),
        pltpu.VMEM((S // 2, Dc), U32),
        pltpu.VMEM((H // 2, Dm, Dh), U32),
        pltpu.VMEM((H // 2, Dc, Dh), U32),
        pltpu.VMEM((H // 2, Dc, Dh), U32),
        pltpu.VMEM((H, Dm // 2, Dh), U32),
        pltpu.VMEM((H, Dh // 2, S), U32),
        pltpu.VMEM((5, S // 4, Dc // 2), U32),
        pltpu.VMEM((2, Dh // 2, Dm), U32),
        pltpu.VMEM((M, Dm), F32),
        pltpu.VMEM((S // 2, Dh), U32),
        pltpu.VMEM((Dh // 2, S), U32),
        pltpu.VMEM((Dm + (-Dm) % 128, S), F32),
        pltpu.VMEM((S, 2 * Dm), BF16),
        pltpu.SemaphoreType.DMA((14, 8)),
    ]
    out = pl.pallas_call(
        kern,
        out_shape=jax.ShapeDtypeStruct((S, 2 * Dm), BF16),
        in_specs=[any_spec] * 12,
        out_specs=any_spec,
        scratch_shapes=scratch,
        compiler_params=pltpu.CompilerParams(vmem_limit_bytes=120 * 1024 * 1024),
    )(A_x[0].T, A_mem0.reshape(M, Dm), A_Wq, A_Wk, A_Wv, jnp.swapaxes(A_Wo, 1, 2),
      B_x[0].T, B_c_kv.reshape(S, Dc), B_w_q, B_w_uk, B_w_uv, jnp.swapaxes(B_w_o, 1, 2))
    return out.reshape(1, S, 2 * Dm)
```

```python
import functools
import jax
import jax.numpy as jnp
import numpy as np
from jax import lax
from jax.experimental import pallas as pl
from jax.experimental.pallas import tpu as pltpu

F32 = jnp.float32
BF16 = jnp.bfloat16
U32 = jnp.uint32

LOG2E = 1.4426950408889634
NEG = -1000000000.0 * LOG2E

KC = 256
EC = 128
RM = 16
RS = 16
KVC = 256
KM = 128
OB = 256

BIAS = 0.005
OPD = 8
TAIL = 2
LAT_S = 150
LAT_O = 450
LAT_R = 200
LAT_M = 150
LAT_BP = 200
LAT_BE = 150
LAT_BO = 350


def _dot(a, b):
    return lax.dot_general(a, b, (((1,), (0,)), ((), ())), preferred_element_type=F32)


def _dot_nt(a, b):
    return lax.dot_general(a, b, (((1,), (1,)), ((), ())), preferred_element_type=F32)


def _unpack(u, shift):
    w = (u << shift) & jnp.uint32(0xFFFF0000)
    return pltpu.bitcast(w, F32).astype(BF16)


def _unpack_f32(u, shift):
    return pltpu.bitcast((u << shift) & jnp.uint32(0xFFFF0000), F32)


def _mo(i, n):
    return i if isinstance(i, int) else pl.multiple_of(i, n)


def _ld(words):
    return pltpu.bitcast(words, BF16)


def _pk(x):
    return pltpu.bitcast(x.astype(BF16), U32)


class _Op:
    def __init__(self, name, cost, deps, fn):
        self.name, self.cost, self.deps, self.fn = name, cost, deps, fn
        self.end = None


def _merge(qa, qb):
    ta = sum(o.cost for o in qa) or 1
    tb = sum(o.cost for o in qb) or 1
    ia = ib = 0
    da = db = 0
    t = 0
    order = []

    def ready(o):
        return max([0] + [d.end + lat for d, lat in o.deps])

    while ia < len(qa) or ib < len(qb):
        cand = []
        if ia < len(qa):
            cand.append((max(ready(qa[ia]), t), da / ta, 0))
        if ib < len(qb):
            cand.append((max(ready(qb[ib]), t), db / tb + BIAS, 1))
        st, _, w = min(cand)
        o = qa[ia] if w == 0 else qb[ib]
        t = st + o.cost
        o.end = t
        order.append(o)
        if w == 0:
            ia += 1
            da += o.cost
        else:
            ib += 1
            db += o.cost
    return order


def _make_kernel(S, Dm, H, Dh, M, seg, Dc):
    n_seg = S // seg
    seg_per_head = n_seg // H
    L = M + seg
    BQ = 128
    nqb = S // BQ
    scale = Dh ** (-0.5) * LOG2E
    PAD = (-Dm) % 128
    LO = Dm + PAD - 128

    def kernel(xat_hbm, mem0_hbm, wq_hbm, wk_hbm, wv_hbm, wot_hbm,
               xbt_hbm, c_hbm, bwq_hbm, wuk_hbm, wuv_hbm, bwot_hbm,
               out_hbm,
               xat, xa, mem0, rq, rk, rv, wkq, wvo, wot,
               xbt, c, rbq, ruk, ruv, bwot,
               qt_all, cs, wqt, memf, kh, vth, acct, outv, sems):

        NP = H // 2

        def pcopy(src, dst, j, s0):
            return pltpu.make_async_copy(src.bitcast(U32).at[:, j, :], dst.at[j], sems.at[s0, j])

        def q_copies(j):
            return [pcopy(bwq_hbm, rbq, j, 0)]

        def a_copies(j):
            return [pcopy(wq_hbm, rq, j, 1), pcopy(wk_hbm, rk, j, 2), pcopy(wv_hbm, rv, j, 3),
                    pltpu.make_async_copy(wot_hbm.bitcast(U32).at[pl.ds(2 * j, 2)], wot.at[pl.ds(2 * j, 2)],
                                          sems.at[9, j])]

        def kv_copies(j):
            return [pcopy(wuk_hbm, ruk, j, 4), pcopy(wuv_hbm, ruv, j, 5)]

        cp_x = pltpu.make_async_copy(xbt_hbm.bitcast(U32), xbt, sems.at[6, 0])
        cp_xa = pltpu.make_async_copy(xat_hbm, xat, sems.at[6, 1])
        cp_m = pltpu.make_async_copy(mem0_hbm, mem0, sems.at[6, 3])
        NL = H // 2
        HL = H // NL

        def c_copies(t):
            n, r = t // (KVC // 256), t % (KVC // 256)
            cps = []
            for half in range(2):
                rows = pl.ds(_mo(n * (KVC // 2) + half * (KVC // 4) + r * 64, 64), 64)
                cps.append(pltpu.make_async_copy(c_hbm.bitcast(U32).at[rows], c.at[rows], sems.at[8 + 5 * half, t]))
            return cps

        def rest_copies(j):
            return [pltpu.make_async_copy(bwot_hbm.bitcast(U32).at[pl.ds(HL * j, HL)], bwot.at[pl.ds(HL * j, HL)],
                                          sems.at[10, j])]

        for cp in q_copies(0) + [cp_x] + q_copies(1):
            cp.start()

        def zero(r, carry):
            acct[:, pl.ds(_mo(r * 128, 128), 128)] = jnp.zeros((acct.shape[0], 128), F32)
            return carry

        lax.fori_loop(0, S // 128, zero, 0)

        def q_weights(h, slot):
            wqt[slot] = _pk(_unpack(rbq[h // 2].T, (16 * (1 - h % 2)).astype(U32)))

        for cp in q_copies(0):
            cp.wait()
        q_weights(jnp.int32(0), 0)
        cp_x.wait()
        cp_xa.start()
        cp_m.start()

        def q_head(h, fill):
            @pl.when((h % 2 == 1) & (h + 1 < H))
            def _():
                for cp in q_copies((h + 1) // 2):
                    cp.wait()

            fill = [functools.partial(q_weights, jnp.minimum(h + 1, H - 1), (h + 1) % 2)] + fill
            nchunk = 8
            cw = S // nchunk
            for n in range(nchunk):
                qt_all[h, :, n * cw:(n + 1) * cw] = _pk(
                    _dot(_ld(wqt[h % 2]), _ld(xbt[:, n * cw:(n + 1) * cw])) * scale)
                for f in fill[len(fill) * n // (nchunk - 1):len(fill) * (n + 1) // (nchunk - 1)]:
                    f()

        KH = KVC // 2
        DH2 = Dc // 2

        def csum(t):
            n, r = t // (KH // 128), t % (KH // 128)
            top = pl.ds(_mo(n * (KVC // 2) + r * 64, 64), 64)
            bot = pl.ds(_mo(n * (KVC // 2) + KH // 2 + r * 64, 64), 64)
            dst = pl.ds(_mo(t * 64, 64), 64)
            blocks = (c[top, 0:DH2], c[top, DH2:], c[bot, 0:DH2], c[bot, DH2:])
            sums = []
            for par in range(2):
                a11, a12, a21, a22 = (_unpack_f32(x, 16 * (1 - par)) for x in blocks)
                sums.append((a11 + a22, a21 + a22, a11 + a12, a21 - a11, a12 - a22))
            for i, (lo, hi) in enumerate(zip(*sums)):
                cs[i, dst, :] = pltpu.bitcast(pltpu.pack_elementwise([lo, hi], packed_dtype=BF16), U32)

        def qproj1(h, carry):
            @pl.when(h + 2 < NP)
            def _():
                for cp in q_copies(h + 2):
                    cp.start()

            @pl.when(h + 2 == NP)
            def _():
                for cp in c_copies(0):
                    cp.start()

            for cp in a_copies(h):
                cp.start()
            q_head(h, [])
            return carry

        def qproj2(j, carry):
            for cp in rest_copies(j):
                cp.start()

            @pl.when(j + 1 < NL)
            def _():
                for cp in c_copies(j + 1):
                    cp.start()

            @pl.when(j == NL // 2)
            def _():
                for cp in kv_copies(0):
                    cp.start()

            for cp in a_copies(j) + c_copies(j):
                cp.wait()

            def side_by_side(dst, ja, lw, rw0, rw1, mul):
                zero = jnp.zeros((PAD, Dh), BF16)
                ev = _dot_nt(_unpack(lw, 16), jnp.concatenate([rw0, zero], axis=0)) * mul
                od = _dot_nt(_unpack(lw, 0), jnp.concatenate([zero, rw1], axis=0)) * mul
                dst[ja, :, 0:LO] = _pk(ev[:, :LO])
                dst[ja, :, LO:LO + 128] = _pk(ev[:, LO:] + od[:, :128])
                dst[ja, :, LO + 128:] = _pk(od[:, 128:])

            def a_vo(ja):
                side_by_side(wvo, ja, rv[ja], _ld(wot[2 * ja]), _ld(wot[2 * ja + 1]), 1.0)

            def a_kq(ja):
                side_by_side(wkq, ja, rk[ja], _unpack(rq[ja], 16), _unpack(rq[ja], 0), scale)

            def tr():
                n = S // NP
                r0 = _mo(j * n, n)
                xa[pl.ds(_mo(j * (n // 2), n // 2), n // 2), :] = _pk(xat[:, pl.ds(r0, n)].T)

            q_head(j + NL, [tr] + [functools.partial(f, j) for f in (csum, a_kq, a_vo)])
            return carry

        lax.fori_loop(0, NL, qproj1, 0)
        cp_xa.wait()
        lax.fori_loop(0, NL, qproj2, 0)

        for j in range(NL):
            for cp in rest_copies(j):
                cp.wait()
        for cp in kv_copies(0) + [cp_m]:
            cp.wait()

        RH = seg_per_head * seg

        def early_out(h):
            r0 = h * RH if isinstance(h, int) else _mo(h * RH, RH)
            return pltpu.make_async_copy(outv.at[pl.ds(r0, RH), pl.ds(0, LO)],
                                         out_hbm.at[pl.ds(r0, RH), pl.ds(0, LO)], sems.at[11 + h // 8, h % 8])

        memf[...] = mem0[...].astype(F32)
        krow = lax.broadcasted_iota(jnp.int32, (BQ, BQ), 0)
        qcol = lax.broadcasted_iota(jnp.int32, (BQ, BQ), 1)
        cmask = krow <= qcol
        GH = 128 // L
        arow = lax.broadcasted_iota(jnp.int32, (L, 128), 0)
        alane = lax.broadcasted_iota(jnp.int32, (L, 128), 1)
        aseg = sum((alane >= L * i).astype(jnp.int32) for i in range(1, GH + 1))
        acol = alane - L * aseg
        amask = (arow < M) | (arow >= acol)
        NPAIR = H // 2
        groups = [list(range(g, min(g + GH, NPAIR))) for g in range(0, NPAIR, GH)]

        def a_ops(s, st, prev):
            r0 = _mo(s * seg, seg)
            v_ = {}

            def f_k(j):
                if j == 0:
                    xs = _ld(xa[pl.ds(_mo(s * (seg // 2), seg // 2), seg // 2), :]).astype(F32)
                    v_["h"] = jnp.concatenate([st["mem"], xs], axis=0)
                    v_["hodd"] = jnp.concatenate([jnp.zeros((L, PAD), F32), v_["h"]], axis=1)
                v_["k", j] = _dot(v_["h"], _ld(wkq[j]))

            def f_u(j):
                v_["u", j] = _dot(v_["h"], _ld(wvo[j]))

            def rows_at(parts):
                used = sum(p.shape[0] for p in parts)
                pad = [jnp.zeros((128 - used, parts[0].shape[1]), F32)]
                return jnp.concatenate(parts + pad, axis=0).astype(BF16)

            def f_s(g, par):
                if par == 0:
                    sc = _dot_nt(v_["h"], rows_at([v_["k", j][:, :Dm] for j in groups[g]]))
                else:
                    ks = [jnp.concatenate([jnp.where(alane < PAD, 0.0, v_["k", j][:, LO:LO + 128]),
                                           v_["k", j][:, LO + 128:]], axis=1) for j in groups[g]]
                    sc = _dot_nt(v_["hodd"], rows_at(ks))
                n = len(groups[g])
                sc = jnp.where(amask & (aseg < n), sc, NEG)
                m = None
                for i in range(n):
                    mi = jnp.max(jnp.where(aseg == i, sc, -jnp.inf), axis=-1, keepdims=True)
                    m = mi if m is None else jnp.where(aseg == i, mi, m)
                p = jnp.where(aseg < n, jnp.exp2(sc - m), 0.0)
                l = None
                for i in range(n):
                    li = jnp.sum(jnp.where(aseg == i, p, 0.0), axis=-1, keepdims=True)
                    l = li if l is None else jnp.where(aseg == i, li, l)
                v_["p", g, par] = p / l

            def f_o(g, par):
                c0 = par * LO
                d = _dot(v_.pop(("p", g, par)), rows_at([v_["u", j][:, c0:c0 + Dm + PAD] for j in groups[g]]))
                v_["acc", par] = d if g == 0 else v_["acc", par] + d
                if g == len(groups) - 1 and par == 1:
                    o = v_["acc", 0][:, :Dm] + v_["acc", 1][:, PAD:]
                    outv[pl.ds(r0, seg), 0:Dm] = o[M:, :].astype(BF16)
                    st["mem"] = o[:M, :]

            P = functools.partial
            kk = [_Op("k%d" % j, 280, [(prev, LAT_M)] if (j == 0 and prev) else [], P(f_k, j)) for j in range(NPAIR)]
            uu = [_Op("u%d" % j, 280, [], P(f_u, j)) for j in range(NPAIR)]
            q = []
            pend = []
            for g, prs in enumerate(groups):
                for j in prs:
                    q.append(kk[j])
                    q += pend
                    pend = []
                q.append(uu[prs[0]])
                ss = [_Op("s", 40, [(kk[prs[-1]], LAT_S)], P(f_s, g, par)) for par in range(2)]
                q += ss
                q += [uu[j] for j in prs[1:]]
                pend = [_Op("o", 40, [(ss[par], LAT_O), (uu[prs[-1]], LAT_R)], P(f_o, g, par)) for par in range(2)]
            return q + pend

        def b_ops(h):
            v_ = {}
            KT = KC // BQ

            def chunks(i):
                return [(t0, min(t0 + KT, i + 1)) for t0 in range(0, i + 1, KT)]

            def f_qk(i, t0, t1):
                qt = _ld(qt_all[h, :, BQ * i:BQ * (i + 1)])
                k0, k1 = BQ * t0, BQ * t1
                km = (k0 + k1) // 2
                sc = jnp.concatenate([_dot(_ld(kh[k0 // 2:km // 2, :]), qt), _dot(_ld(kh[km // 2:k1 // 2, :]), qt)], axis=0)
                if t1 == i + 1:
                    sd = jnp.where(cmask, sc[k1 - k0 - BQ:, :], NEG)
                    sc = jnp.concatenate([sc[:k1 - k0 - BQ, :], sd], axis=0) if t1 - t0 > 1 else sd
                v_["s", i, t0] = sc
                m = jnp.max(sc.reshape((k1 - k0) // RM, RM, BQ), axis=0)
                v_["m", i] = m if t0 == 0 else jnp.maximum(v_["m", i], m)
                if t1 == i + 1:
                    v_["m", i] = jnp.max(v_["m", i], axis=0, keepdims=True)

            def f_e(i, t0, t1, e0, e1):
                p = jnp.exp2(v_["s", i, t0][e0:e1, :] - v_["m", i])
                l = jnp.sum(p.reshape((e1 - e0) // RS, RS, BQ), axis=0)
                v_["l", i] = l if (t0 == 0 and e0 == 0) else v_["l", i] + l
                v_.setdefault(("p", i, t0), []).append(p.astype(BF16))

            def f_pv(i, t0, t1):
                p = jnp.concatenate(v_.pop(("p", i, t0)), axis=0)
                ns = {0: 1, 1: 4, 2: 2, 3: 4}[(t1 - t0) % 4]
                rr = Dh // ns
                d = jnp.concatenate([_dot(_ld(vth[r * rr // 2:(r + 1) * rr // 2, BQ * t0:BQ * t1]), p) for r in range(ns)], axis=0)
                v_["c", i] = d if t0 == 0 else v_["c", i] + d
                if t1 == i + 1:
                    r = 1.0 / jnp.sum(v_.pop(("l", i)), axis=0, keepdims=True)
                    v_["c", i] = v_["c", i] * r

            hm = Dm // 2

            def f_wo():
                w = _ld(bwot[h]).astype(F32)
                w11, w12, w21, w22 = w[:hm, :128], w[:hm, 128:], w[hm:, :128], w[hm:, 128:]
                v_["wo"] = [x.astype(BF16)
                            for x in (w11 + w22, w21 + w22, w11, w22, w11 + w12, w21 - w11, w12 - w22)]

            def f_op(i):
                c0, c1 = v_.pop(("c", i)), v_.pop(("c", i + 1))
                cc = wcombos(c0[:128], c1[:128], c0[128:], c1[128:])
                o11, o12, o21, o22 = outs([_dot(v_["wo"][p], cc[p]) for p in range(7)])
                acct[PAD:PAD + hm, BQ * i:BQ * (i + 1)] += o11
                acct[PAD:PAD + hm, BQ * (i + 1):BQ * (i + 2)] += o12
                acct[PAD + hm:, BQ * i:BQ * (i + 1)] += o21
                acct[PAD + hm:, BQ * (i + 1):BQ * (i + 2)] += o22

            shift = (16 * (1 - h % 2)).astype(U32)

            def wcombos(w11, w12, w21, w22):
                return [x.astype(BF16) for x in (w11 + w22, w11, w12 - w22, w21 - w11, w22, w11 + w12, w21 + w22)]

            def lhs(p, n, r):
                if p == 2:
                    return _ld(c[(n * KVC + r) // 2:(n * KVC + r + KM) // 2, 0:DH2])
                if p == 3:
                    return _ld(c[(n * KVC + KH + r) // 2:(n * KVC + KH + r + KM) // 2, DH2:])
                return _ld(cs[(0, 1, None, None, 2, 3, 4)[p], (n * KH + r) // 2:(n * KH + r + KM) // 2, :])

            def outs(m):
                return (m[0] + m[3] - m[4] + m[6], m[2] + m[4], m[1] + m[3], m[0] - m[1] + m[2] + m[5])

            def f_kp(n, r):
                if "wk" not in v_:
                    w = _unpack_f32(ruk[h // 2], shift)
                    v_["wk"] = wcombos(w[:DH2, :128], w[:DH2, 128:], w[DH2:, :128], w[DH2:, 128:])
                c11, c12, c21, c22 = outs([_dot(lhs(p, n, r), v_["wk"][p]) for p in range(7)])
                top = slice((n * KVC + r) // 2, (n * KVC + r + KM) // 2)
                bot = slice((n * KVC + KH + r) // 2, (n * KVC + KH + r + KM) // 2)
                kh[top, 0:128] = _pk(c11)
                kh[top, 128:] = _pk(c12)
                kh[bot, 0:128] = _pk(c21)
                kh[bot, 128:] = _pk(c22)

            def f_vp(n, r):
                if "wv" not in v_:
                    w = _unpack_f32(ruv[h // 2].T, shift)
                    v_["wv"] = wcombos(w[:128, :DH2], w[128:, :DH2], w[:128, DH2:], w[128:, DH2:])
                c11, c12, c21, c22 = outs([_dot_nt(v_["wv"][p], lhs(p, n, r)) for p in range(7)])
                top = slice(n * KVC + r, n * KVC + r + KM)
                bot = slice(n * KVC + KH + r, n * KVC + KH + r + KM)
                vth[0:64, top] = _pk(c11)
                vth[64:, top] = _pk(c12)
                vth[0:64, bot] = _pk(c21)
                vth[64:, bot] = _pk(c22)

            P = functools.partial
            nr = [(n, r) for n in range(S // KVC) for r in range(0, KH, KM)]
            kp = [_Op("K", 7 * KM, [], P(f_kp, n, r)) for n, r in nr]
            vp = [_Op("V", 7 * KM, [], P(f_vp, n, r)) for n, r in nr]
            qk = [[_Op("QK%d" % i, 64 * (t1 - t0), [], P(f_qk, i, t0, t1)) for t0, t1 in chunks(i)]
                  for i in range(nqb)]
            epv = []
            for i in range(nqb):
                es = [[_Op("E", 0, [(qk[i][-1], LAT_BP)], P(f_e, i, t0, t1, e0, min(e0 + EC, BQ * (t1 - t0))))
                       for e0 in range(0, BQ * (t1 - t0), EC)] for t0, t1 in chunks(i)]
                pv = [_Op("PV%d" % i, 64 * (t1 - t0), [(es[n][-1], LAT_BE)], P(f_pv, i, t0, t1))
                      for n, (t0, t1) in enumerate(chunks(i))]
                l = list(es[0])
                for n in range(len(pv)):
                    if n + 1 < len(pv):
                        l += es[n + 1]
                    l.append(pv[n])
                epv.append(l)
            op = {i: _Op("OP%d" % i, 392, [(epv[i][-1], LAT_BO), (epv[i + 1][-1], LAT_BO)], P(f_op, i)) for i in range(0, nqb, 2)}
            q = kp[:4] + [_Op('W', 0, [], f_wo)] + kp[4:] + vp[:1]
            order = list(range(nqb - 1, -1, -1))
            for t in range(nqb + OPD):
                l1 = qk[order[t]] if t < nqb else []
                l2 = epv[order[t - 1]] if 0 <= t - 1 < nqb else (vp[1:] if t == 0 else [])
                keyed = [((n + 0.25) / len(l1), 0, o) for n, o in enumerate(l1)]
                keyed += [((n + 0.75) / len(l2), 1, o) for n, o in enumerate(l2)]
                q += [o for _, _, o in sorted(keyed, key=lambda z: z[:2])]
                if 0 <= t - OPD < nqb and (t - OPD) % 2 == 1:
                    q.append(op[order[t - OPD] // 2 * 2])
            return q

        def head(h, carry):
            @pl.when((h % 2 == 0) & (h < H - 2))
            def _():
                for cp in kv_copies(h // 2 + 1):
                    cp.start()

            @pl.when((h % 2 == 1) & (h < H - 1))
            def _():
                for cp in kv_copies(h // 2 + 1):
                    cp.wait()

            @pl.when(h > 0)
            def _():
                early_out(h - 1).start()

            st = {"mem": memf[...]}
            qa = []
            for t in range(seg_per_head):
                qa += a_ops(h * seg_per_head + t, st, qa[-1] if qa else None)
            qb = b_ops(h)
            nb = len(qb) - TAIL
            for o in _merge(qa, qb[:nb]) + qb[nb:]:
                o.fn()
            memf[...] = st["mem"]
            return carry

        lax.fori_loop(0, H, head, 0)

        def out_copy(r):
            r0 = _mo(r * OB, OB)
            return pltpu.make_async_copy(outv.at[pl.ds(r0, OB), pl.ds(LO, 2 * Dm - LO)],
                                         out_hbm.at[pl.ds(r0, OB), pl.ds(LO, 2 * Dm - LO)], sems.at[7, r])

        def epi(r, carry):
            lane = lax.broadcasted_iota(jnp.int32, (OB, 128), 1)
            rows = pl.ds(_mo(r * OB, OB), OB)
            bt = acct[:, rows].T.astype(BF16)
            outv[rows, LO:LO + 128] = jnp.where(lane < 128 - PAD, outv[rows, LO:LO + 128], bt[:, 0:128])
            outv[rows, LO + 128:] = bt[:, 128:]
            out_copy(r).start()
            return carry

        early_out(H - 1).start()
        lax.fori_loop(0, S // OB, epi, 0)
        for hh in range(H):
            early_out(hh).wait()
        for r in range(S // OB):
            out_copy(r).wait()

    return kernel


@functools.partial(jax.jit, static_argnames=("A_seg_len",))
def pallas_concat_heads__memory_aug_recurrent_mem_tr__compressed_kv_cla__prompt_kernel(A_x, A_mem0, A_Wq, A_Wk, A_Wv, A_Wo, A_seg_len, B_x, B_c_kv, B_w_q, B_w_uk, B_w_uv, B_w_o):
    _, S, Dm = A_x.shape
    M = A_mem0.shape[1]
    H, Dh = A_Wq.shape[1], A_Wq.shape[2]
    Dc = B_c_kv.shape[2]
    seg = int(A_seg_len)
    kern = _make_kernel(S, Dm, H, Dh, M, seg, Dc)
    any_spec = pl.BlockSpec(memory_space=pl.ANY)
    scratch = [
        pltpu.VMEM((Dm, S), BF16),
        pltpu.VMEM((S // 2, Dm), U32),
        pltpu.VMEM((M, Dm), BF16),
        pltpu.VMEM((H // 2, Dm, Dh), U32),
        pltpu.VMEM((H // 2, Dm, Dh), U32),
        pltpu.VMEM((H // 2, Dm, Dh), U32),
        pltpu.VMEM((H // 2, Dm // 2, 2 * Dm), U32),
        pltpu.VMEM((H // 2, Dm // 2, 2 * Dm), U32),
        pltpu.VMEM((H, Dm // 2, Dh), U32),
        pltpu.VMEM((Dm // 2, S), U32),
        pltpu.VMEM((S // 2, Dc), U32),
        pltpu.VMEM((H // 2, Dm, Dh), U32),
        pltpu.VMEM((H // 2, Dc, Dh), U32),
        pltpu.VMEM((H // 2, Dc, Dh), U32),
        pltpu.VMEM((H, Dm // 2, Dh), U32),
        pltpu.VMEM((H, Dh // 2, S), U32),
        pltpu.VMEM((5, S // 4, Dc // 2), U32),
        pltpu.VMEM((2, Dh // 2, Dm), U32),
        pltpu.VMEM((M, Dm), F32),
        pltpu.VMEM((S // 2, Dh), U32),
        pltpu.VMEM((Dh // 2, S), U32),
        pltpu.VMEM((Dm + (-Dm) % 128, S), F32),
        pltpu.VMEM((S, 2 * Dm), BF16),
        pltpu.SemaphoreType.DMA((14, 8)),
    ]
    out = pl.pallas_call(
        kern,
        out_shape=jax.ShapeDtypeStruct((S, 2 * Dm), BF16),
        in_specs=[any_spec] * 12,
        out_specs=any_spec,
        scratch_shapes=scratch,
        compiler_params=pltpu.CompilerParams(vmem_limit_bytes=120 * 1024 * 1024),
    )(A_x[0].T, A_mem0.reshape(M, Dm), A_Wq, A_Wk, A_Wv, jnp.swapaxes(A_Wo, 1, 2),
      B_x[0].T, B_c_kv.reshape(S, Dc), B_w_q, B_w_uk, B_w_uv, jnp.swapaxes(B_w_o, 1, 2))
    return out.reshape(1, S, 2 * Dm)
```
